```python
import os as _os
_os.environ.setdefault("JAX_PLATFORMS", "cpu")
import jax
import jax.numpy as jnp

def _softmax(x, axis=-1):
    return jax.nn.softmax(x, axis=axis)
def _gelu(x):
    return jax.nn.gelu(x, approximate=True)
def _silu(x):
    return jax.nn.silu(x)
def _sigmoid(x):
    return jax.nn.sigmoid(x)
def _layernorm(x, axis=-1, eps=1e-5):
    m = jnp.mean(x, axis=axis, keepdims=True)
    v = jnp.var(x, axis=axis, keepdims=True)
    return (x - m) / jnp.sqrt(v + eps)
def _scatter_add(tgt, idx, src, axis=0):
    return tgt.at[idx].add(src)
def _segment_sum(src, seg, n):
    return jax.ops.segment_sum(src, seg, n)
class _Rng:
    def __init__(self, key):
        self._k = key
    def _next(self):
        self._k, sub = jax.random.split(self._k)
        return sub
    def normal(self, shape):
        return jax.random.normal(self._next(), shape, dtype=jnp.bfloat16)
    def randint(self, lo, hi, shape):
        return jax.random.randint(self._next(), shape, lo, hi, dtype=jnp.int32)
    def uniform(self, shape, lo=0.0, hi=1.0):
        return jax.random.uniform(self._next(), shape, jnp.bfloat16, lo, hi)
    def permutation(self, n):
        return jax.random.permutation(self._next(), n)


kernel_name = 'sequential_preLN__sliding_block__dense_activation_relu__prompt'

def setup_inputs():
    _rng = _Rng(jax.random.key(int.from_bytes(__import__("os").urandom(4), "little")))
    _w = (lambda a: (lambda t: t.astype(jnp.bfloat16) if jnp.issubdtype(t.dtype, jnp.floating) else t)(jnp.asarray(a)))
    def _A_setup():
        B, S, D = 1, 2048, 640
        return {
            "x": _w((lambda *s: _rng.normal(s) * 0.05)(B, S, D)),
            "wqkv": _w((lambda *s: _rng.normal(s) * 0.05)(D, 3 * D)),
            "wo": _w((lambda *s: _rng.normal(s) * 0.05)(D, D)),
        }
    _A_in = _A_setup()

    def _B_setup():
        B, S, D, Dff = 1, 2048, 640, 1536
        return {
            "x": _w((lambda *s: _rng.normal(s) * 0.05)(B, S, D)),
            "w1": _w((lambda *s: _rng.normal(s) * 0.05)(D, Dff)),
            "w2": _w((lambda *s: _rng.normal(s) * 0.05)(Dff, D)),
        }
    _B_in = _B_setup()

    return {
        "A_x": _A_in["x"],
        "A_wqkv": _A_in["wqkv"],
        "A_wo": _A_in["wo"],
        "B_x": _B_in["x"],
        "B_w1": _B_in["w1"],
        "B_w2": _B_in["w2"],
    }

def reference(A_x, A_wqkv, A_wo, B_x, B_w1, B_w2):
    def _A_ref(x, wqkv, wo):
        B, S, D = x.shape
        H = 32; Dh = D // H; W = 256
        qkv = (lambda x, *d: x.transpose(*d))((x @ wqkv).reshape(B, S, 3, H, Dh), 2, 0, 3, 1, 4)
        q, k, v = qkv[0], qkv[1], qkv[2]
        scores = jnp.einsum("bhqd,bhkd->bhqk", q, k) * (Dh ** -0.5)
        idx = jnp.arange(S)
        mask = (idx[:, None] - idx[None, :] >= 0) & (idx[:, None] - idx[None, :] < W)
        scores = jnp.where(mask[None, None], scores, -1e9)
        p = _softmax(scores, axis=-1)
        o = jnp.einsum("bhqk,bhkd->bhqd", p, v)
        return (lambda x, *d: x.transpose(*d))(o, 0, 2, 1, 3).reshape(B, S, D) @ wo

    def _B_ref(x, w1, w2):
        h = jnp.einsum("bsd,df->bsf", x, w1)
        zero = jnp.zeros_like(h)
        h = jnp.maximum(h, zero)
        return jnp.einsum("bsf,fd->bsd", h, w2)

    x = A_x
    h = x + _A_ref(_layernorm(x, axis=-1), A_wqkv, A_wo)
    h2 = h + _B_ref(_layernorm(h, axis=-1), B_w1, B_w2)
    return h2
```

```python
import functools
import jax
import jax.numpy as jnp
import numpy as np
from jax import lax
from jax.experimental import pallas as pl
from jax.experimental.pallas import tpu as pltpu

NN = (((1,), (0,)), ((), ()))
NT = (((1,), (1,)), ((), ()))
BF, F32, U32, I32 = jnp.bfloat16, jnp.float32, jnp.uint32, jnp.int32
H, DH, W = 32, 20, 256
EPS = 1e-5
QSCALE = float(DH ** -0.5 * np.log2(np.e))


def _mm(a, b, dn=NN):
    return lax.dot_general(a, b, dn, preferred_element_type=F32)


def _ln(x):
    d = x.shape[-1]
    m = jnp.sum(x, axis=-1, keepdims=True) * (1.0 / d)
    c = x - m
    v = jnp.sum(c * c, axis=-1, keepdims=True) * (1.0 / d)
    return c * lax.rsqrt(v + EPS)


def _kernel(x_hbm, wqkv_hbm, wo_hbm, w1_hbm, w2_hbm, out_hbm,
            x_s, wqkv_s, wo_s, w1_s, w2_s, wqvt_s, qt_s, k_s, vt_s, o_s, out_s, sem_in, sem_x, sem_out,
            *, S, D, TA, TC, lag):
    nA, nC = S // TA, S // TC
    x_cp = [pltpu.make_async_copy(x_hbm.at[pl.ds(i * TA, TA)], x_s.at[pl.ds(i * TA, TA)], sem_x.at[i]) for i in range(nA)]
    w_cp = [pltpu.make_async_copy(s, d, sem_in.at[i]) for i, (s, d) in enumerate(
        [(wqkv_hbm, wqkv_s), (wo_hbm, wo_s), (w1_hbm, w1_s), (w2_hbm, w2_s)])]
    x_cp[0].start()
    w_cp[0].start()
    for c in x_cp[1:]:
        c.start()
    for c in w_cp[1:]:
        c.start()
    w_cp[0].wait()
    wqvt_s[0:D, :] = wqkv_s[:, 0:D].astype(F32).T.astype(BF)
    wqvt_s[D:2 * D, :] = wqkv_s[:, 2 * D:3 * D].astype(F32).T.astype(BF)
    for c in x_cp:
        c.wait()

    sub = lax.broadcasted_iota(I32, (8, 128), 0)

    def phase_a(i, carry):
        r0 = pl.multiple_of(i * TA, TA)
        xn = _ln(x_s[pl.ds(r0, TA), :].astype(F32)).astype(BF)
        k_s[pl.ds(r0, TA), :] = _mm(xn, wqkv_s[:, D:2 * D]).astype(BF)
        qv = _mm(wqvt_s[...], xn, NT)
        qt_s[:, pl.ds(r0, TA)] = (qv[0:D] * QSCALE).astype(BF)
        subw = lax.broadcasted_iota(I32, (8, TA), 0)
        for p in range(H // 2):
            v = qv[D + 40 * p:D + 40 * p + 40]
            mid = v[16:24]
            vt_s[48 * p:48 * p + 48, pl.ds(r0, TA)] = jnp.concatenate(
                [v[0:16], jnp.where(subw < 4, mid, 1.0), jnp.where(subw < 4, 1.0, mid), v[24:40]], axis=0)
        return carry

    lax.fori_loop(0, nA, phase_a, 0)

    def attn_block(qb, nk):
        r0 = qb * 128 if isinstance(qb, int) else pl.multiple_of(qb * 128, 128)
        k0 = r0 - 128 * (nk - 1)
        if not isinstance(qb, int):
            k0 = pl.multiple_of(k0, 128)
        tri = lax.broadcasted_iota(I32, (128, 128), 0) <= lax.broadcasted_iota(I32, (128, 128), 1)
        lane_k = lax.broadcasted_iota(I32, (64 * nk, 128), 1)

        def qk(h):
            lo, hi = DH * h, DH * h + DH
            t0, t1 = lo // 128, (hi - 1) // 128
            if t0 == t1:
                k = k_s[pl.ds(k0, 128 * nk), t0 * 128:(t0 + 1) * 128]
            else:
                ka = pltpu.bitcast(k_s[pl.ds(k0, 128 * nk), t0 * 128:(t0 + 1) * 128], U32)
                kb = pltpu.bitcast(k_s[pl.ds(k0, 128 * nk), t1 * 128:(t1 + 1) * 128], U32)
                k = pltpu.bitcast(jnp.where(lane_k < 64, kb, ka), BF)
            tiles = [None] * 8
            for j in range(lo // 16, (hi - 1) // 16 + 1):
                q = pltpu.bitcast(qt_s[16 * j:16 * j + 16, pl.ds(r0, 128)], U32)
                a, b = (lo - 16 * j) // 2, (hi - 16 * j) // 2
                if a > 0:
                    q = jnp.where(sub >= a, q, jnp.uint32(0))
                if b < 8:
                    q = jnp.where(sub < b, q, jnp.uint32(0))
                tiles[j % 8] = q
            z = jnp.zeros((8, 128), U32)
            wq = pltpu.bitcast(jnp.concatenate([z if t is None else t for t in tiles], axis=0), BF)
            return _mm(k, wq)

        def softmax(s):
            if nk == 3:
                sm, sf = jnp.where(tri, s[256:384], s[0:128]), s[128:256]
            elif nk == 2:
                sm, sf = jnp.where(tri, s[128:256], -jnp.inf), s[0:128]
            else:
                sm, sf = jnp.where(tri, s, -jnp.inf), None
            mx = jnp.max(sm if sf is None else jnp.maximum(sm, sf), axis=0, keepdims=True)
            pm = jnp.exp2(sm - mx)
            if nk == 1:
                return [pm]
            pf = jnp.exp2(sf - mx)
            if nk == 2:
                return [pf, pm]
            return [jnp.where(tri, 0.0, pm), pf, jnp.where(tri, pm, 0.0)]

        def pv(h, p):
            v = vt_s[24 * h:24 * h + 24, pl.ds(k0, 128 * nk)]
            return _mm(v, jnp.concatenate(p, axis=0).astype(BF))

        G = 4
        ng = H // G
        Sc, O, rows = {}, {}, []
        for step in range(ng + lag):
            if step < ng:
                for h in range(step * G, step * G + G):
                    Sc[h] = qk(h)
            g = step - lag
            if g >= 0:
                P = {h: softmax(Sc.pop(h)) for h in range(g * G, g * G + G)}
                for h in range(g * G, g * G + G):
                    O[h] = pv(h, P[h])
                for h in range(g * G + 1, g * G + G, 2):
                    e, o = O.pop(h - 1), O.pop(h)
                    l = jnp.where(sub < 4, o[0:8], e[16:24])
                    r = pltpu.reciprocal(l, approx=True)
                    r = r * (2.0 - l * r)
                    e, o = e * r[4:5], o * r[0:1]
                    rows += [e[0:16], jnp.where(sub < 4, e[16:24], o[0:8]), o[8:24]]
        ot = jnp.concatenate(rows, axis=0)
        o_s[pl.ds(r0, 128), :] = ot.T.astype(BF)

    attn_block(0, 1)
    attn_block(1, 2)

    def phase_b(i, carry):
        attn_block(i, 3)
        return carry

    lax.fori_loop(2, S // 128, phase_b, 0)

    for c in w_cp[1:]:
        c.wait()

    def phase_c(i, carry):
        r0 = pl.multiple_of(i * TC, TC)
        h = x_s[pl.ds(r0, TC), :].astype(F32) + _mm(o_s[pl.ds(r0, TC), :], wo_s[...])
        hn = _ln(h).astype(BF)
        a = jnp.maximum(_mm(hn, w1_s[...]), 0.0).astype(BF)
        out_s[pl.ds(r0, TC), :] = (h + _mm(a, w2_s[...])).astype(BF)
        pltpu.make_async_copy(out_s.at[pl.ds(r0, TC)], out_hbm.at[pl.ds(r0, TC)], sem_out.at[i]).start()
        return carry

    lax.fori_loop(0, nC, phase_c, 0)
    for i in range(nC):
        pltpu.make_async_copy(out_s.at[pl.ds(i * TC, TC)], out_hbm.at[pl.ds(i * TC, TC)], sem_out.at[i]).wait()


def make(TA=256, TC=256, lag=3):
    def fn(A_x, A_wqkv, A_wo, B_x, B_w1, B_w2):
        del B_x
        B, S, D = A_x.shape
        F = B_w1.shape[1]
        anyspec = pl.BlockSpec(memory_space=pl.ANY)
        out = pl.pallas_call(
            functools.partial(_kernel, S=S, D=D, TA=TA, TC=TC, lag=lag),
            in_specs=[anyspec] * 5,
            out_specs=anyspec,
            out_shape=jax.ShapeDtypeStruct((S, D), A_x.dtype),
            scratch_shapes=[
                pltpu.VMEM((S, D), BF), pltpu.VMEM((D, 3 * D), BF), pltpu.VMEM((D, D), BF),
                pltpu.VMEM((D, F), BF), pltpu.VMEM((F, D), BF),
                pltpu.VMEM((2 * D, D), BF), pltpu.VMEM((D, S), BF), pltpu.VMEM((S, D), BF),
                pltpu.VMEM((24 * H, S), F32), pltpu.VMEM((S, D), BF), pltpu.VMEM((S, D), BF),
                pltpu.SemaphoreType.DMA((4,)), pltpu.SemaphoreType.DMA((S // TA,)), pltpu.SemaphoreType.DMA((S // TC,)),
            ],
            compiler_params=pltpu.CompilerParams(vmem_limit_bytes=100 << 20),
            name="fused_layer",
        )(A_x.reshape(S, D), A_wqkv, A_wo, B_w1, B_w2)
        return out.reshape(B, S, D)
    return fn


@jax.jit
def pallas_sequential_preLN__sliding_block__dense_activation_relu__prompt_kernel(
    A_x: jax.Array,
    A_wqkv: jax.Array,
    A_wo: jax.Array,
    B_x: jax.Array,
    B_w1: jax.Array,
    B_w2: jax.Array,
):
    return make()(A_x, A_wqkv, A_wo, B_x, B_w1, B_w2)
```

```python
import functools
import heapq

import jax
import jax.numpy as jnp
import numpy as np
from jax import lax
from jax.experimental import pallas as pl
from jax.experimental.pallas import tpu as pltpu

BF, F32, U32, I32 = jnp.bfloat16, jnp.float32, jnp.uint32, jnp.int32
H, DH = 32, 20
NG = H // 4
TB = 256
HB = TB // 2
RB, RH = TB // 2, HB // 2
SPARE = 8
EPS = 1e-5
QSCALE = float(DH ** -0.5 * np.log2(np.e))

_PACE = dict(chunk=16, turns=1, even=1.5, after=300, exp=(192, 96), o_first=288, o_after=600, o_span=1000,
             q_span=900, v_span=1000, pin_stats=True, norm=((0, 1, 2),), hold_ln1=(512, 224), hold_ln2=(512, 256),
             hold_skew=224, skew_cuts=(2, 4))
_PACES = dict(
    start0=dict(),
    start1=dict(chunk=32, turns=4, t=((0.02, 0.4), (0.1, 0.4), (0.5, 0.95), (0.6, 0.9))),
    start2=dict(chunk=32, v_span=800, pin_stats=False, hold_ln1=(400, 224), norm=((0,), (1, 2)),
                skew_cuts=(1, 2, 3, 4), t=((0.01, 0.3), (0.04, 0.14), (0.18, 0.38), (0.7, 0.95), (0.4, 0.7))),
    proj=dict(chunk=32, after=400, q_span=600, v_span=800, pin_stats=False, hold_ln1=(400, 224),
              norm=((0,), (1, 2)), skew_cuts=(1, 2, 3, 4), t=((0.04, 0.14), (0.18, 0.38), (0.5, 0.8), (0.15, 0.66))),
    attn0=dict(exp=(224, 96), q_span=1200, v_span=1200, norm=((0,), (1,), (2,)), share=0.33,
               t=((0.02, 0.97), (0.04, 0.12), (0.14, 0.3), (0.3, 0.64), (0.03, 0.08), (0.12, 0.3), (0.33, 0.6))),
    attn1=dict(chunk=32, turns=2, even=5, q_span=2400, v_span=3000, skew_cuts=(1, 2, 3, 4), ln_span=2400,
               skew_span=5000, t=((0.01, 0.33), (0.02, 0.97))),
    main=dict(cut=44, ln_span=2200),
    finish=dict(cut=(40, 100), ln_span=1500),
)


def _mm(a, b):
    return lax.dot_general(a, b, (((1,), (0,)), ((), ())), preferred_element_type=F32)


def _iota(shape, d):
    return lax.broadcasted_iota(I32, shape, d)


def _at(start, n, multiple):
    return pl.ds(start if isinstance(start, int) else pl.multiple_of(start, multiple), n)


def _u32(x):
    return pltpu.bitcast(x, U32)


def _bf(x):
    return pltpu.bitcast(x, BF)


def _pack(x):
    return _u32(x.astype(BF))


def _col(c, n=1):
    return slice(128 * c, 128 * (c + n))


def _tile(i, rows, r, n):
    return slice(i // 4 * rows + r, i // 4 * rows + r + n), _col(i % 4)


def _left_terms(a11, a12, a21, a22):
    return [a11 + a22, a21 + a22, a11, a22, a11 + a12, a21 - a11, a12 - a22, a12, a21]


def _right_terms(b11, b12, b21, b22):
    return [b11 + b22, b11, b12 - b22, b21 - b11, b22, b11 + b12, b21 + b22]


_QUADRANT = ((2, 7), (8, 3))


def _choose_cuts(jobs, n, even):
    rounds = (len(jobs) + 3) // 4
    open_at = [0] + [jobs[min(4 * r, len(jobs)) - 1][4] for r in range(1, rounds + 1)]
    best = {0: (0.0, [0])}
    for _ in range(n):
        best = {r: min((cost + open_at[r] + even * (r - p - rounds / n) ** 2, path + [r])
                       for p, (cost, path) in best.items() if p < r)
                for r in range(min(best) + 1, rounds + 1)}
    return best[rounds][1]


class _Timeline:
    def __init__(self, pin, chunk, turns):
        self.pin, self.chunk, self.turns = pin, chunk, turns
        self.t = self.now = self.count = self.turn = 0
        self.queue, self.stored, self.results = [], {}, []

    def spread(self, t0, t1, tasks, key=None):
        for i, task in enumerate(tasks):
            if task is not None:
                heapq.heappush(self.queue, (t0 + (t1 - t0) * i / max(len(tasks) - 1, 1), self.count, task, key))
                self.count += 1

    def run(self, t):
        self.now = t
        while self.queue and self.queue[0][0] <= t:
            ref = heapq.heappop(self.queue)[2]()
            if ref is not None:
                self.stored[id(ref)] = ref

    def need(self, keys):
        due = sorted(e for e in self.queue if e[3] in keys)
        self.queue = [e for e in self.queue if e[3] not in keys]
        heapq.heapify(self.queue)
        for e in due:
            e[2]()

    def hold(self, ref, lag):
        old = [v for t, v in self.results if t <= self.now - lag]
        if old:
            ref[ref.shape[0] - SPARE:, _col(0)] = old[-1] if ref.dtype == F32 else _u32(old[-1])

    def round(self, jobs, rows):
        parts = [[] for _ in jobs]
        self.need({k for job in jobs for k in job[3]})
        for r in range(0, rows, self.chunk):
            self.run(self.t + r)
            for p, job in zip(parts, jobs):
                p.append(job[0](r, self.chunk))
            for ref in self.stored.values():
                self.turn = (self.turn + 1) % self.turns
                parts[self.turn][-1] = self.pin(parts[self.turn][-1], ref)
            self.stored = {}
        for p, job in zip(parts, jobs):
            res = _mm(_bf(jnp.concatenate(p, axis=0)), job[1]())
            out = job[2](res)
        out = res if out is None else out
        self.results += [(self.t + r, out[r:r + SPARE]) for r in range(0, rows, self.chunk)]
        self.t += rows


def _kernel(x_hbm, wqkv_hbm, wo_hbm, w1_hbm, w2_hbm, out_hbm,
            x_s, wqkv_s, wo_s, w1_s, w2_s, cqkv_s, co_s, c1_s, c2_s, ln1_s, ln2_s, xn_s, q_s, v_s, vp_s,
            qt_s, k_s, ks_s, vt_s, s_s, p_s, ot_s, o_s, h_s, hn_s, a_s, out_s, sem_w, sem_x, sem_out):
    (S, D), FF = x_hbm.shape, w1_hbm.shape[1]
    NB, ND, NF = S // TB, D // 128, FF // 128
    KH, FH = ND // 2, NF // 2
    XR = o_s.shape[0] - SPARE
    cur = {}

    def pace(name):
        cur.update(_PACE, **_PACES[name])

    def x_cp(i):
        return pltpu.make_async_copy(x_hbm.at[pl.ds(i * TB, TB)], x_s.at[pl.ds(i * TB, TB)], sem_x.at[i])

    def out_cp(i, c0=0, c1=ND):
        at = (_at(i * TB, TB, TB), pl.ds(128 * c0, 128 * (c1 - c0)))
        return pltpu.make_async_copy(out_s.at[at], out_hbm.at[at], sem_out.at[i + (c0 > 0)])

    head = 3
    wq_head, wq_rest, wk_cp, wv_cp = [
        pltpu.make_async_copy(wqkv_hbm.at[:, pl.ds(c0, c1 - c0)], wqkv_s.at[:, pl.ds(c0, c1 - c0)], sem_w.at[i])
        for i, (c0, c1) in enumerate(((0, 128 * head), (128 * head, D), (D, 2 * D), (2 * D, 3 * D)))]
    late_cps = [pltpu.make_async_copy(src, dst, sem_w.at[4 + i])
                for i, (src, dst) in enumerate(((wo_hbm, wo_s), (w1_hbm, w1_s), (w2_hbm, w2_s)))]
    for cp in (x_cp(0), wq_head, x_cp(1), wq_rest):
        cp.start()

    k_s[0:48, :] = jnp.zeros((48, D), U32)
    for ref in (*cqkv_s, co_s, c1_s, c2_s, *ln1_s, *ln2_s, xn_s, vp_s, qt_s, ks_s, vt_s, *p_s, o_s, hn_s):
        ref[ref.shape[0] - SPARE:, _col(0)] = jnp.zeros((SPARE, 128), ref.dtype)

    zero = lax.fori_loop(0, 2, lambda i, c: i * (i - 1) * (2 * i - 1) * 128, jnp.int32(0))
    keep = _iota((8, 128), 0) >= zero

    def dyn(ref, row=0, n=None, multiple=8):
        return ref.at[_at(zero + row, n or ref.shape[0], multiple)]

    def pin(v, ref):
        n = 2 * SPARE if ref.dtype == BF else SPARE
        w = dyn(ref, multiple=n)[ref.shape[0] - n:, _col(0)]
        first = jnp.where(keep, v[0:8], w if w.dtype == U32 else _u32(w))
        return jnp.concatenate([first, v[8:]], axis=0) if v.shape[0] > 8 else first

    def chain(n, lhs, rhs, key, start, finish, live=(1, 0)):
        acc = []

        def done(r):
            prev = acc[-1] if acc else start()
            acc.append(r if prev is None else r + prev)
            if len(acc) == n:
                finish(acc[-1])
            return acc[-1]
        return [(functools.partial(lhs, k), functools.partial(rhs, k), done, key(k), live[k == n - 1])
                for k in range(n)]

    def gemm_jobs(a_ref, row0, rows, tag, c_ref, nk, nn, done, key=lambda k: (), held=0):
        kh, nh, odd = nk // 2, nn // 2, nk % 2
        none = lambda: None

        def left(c, term, k, r, n):
            return dyn(a_ref, row0 + (tag + c) * zero, rows)[_tile(term * kh + k, RH, r // 2, n // 2)]

        def plain_left(c, half, k, r, n):
            if k < 2 * kh:
                return left(c, _QUADRANT[half][k // kh], k % kh, r, n)
            return left(c, 9, half, r, n)

        def right(i):
            return _bf(dyn(c_ref)[_tile(i, 64, 0, 64)])

        jobs = []
        for c in range(nh):
            v = {}

            def prod(term, start, finish, live, c=c):
                return chain(kh, functools.partial(left, c, term), lambda k: right((term * kh + k) * nh + c),
                             lambda k: key(k) + key(kh + k), start, finish, live)

            def rest(half, cc, start, finish, live):
                return chain(odd, lambda k, r, n: plain_left(cc, half, 2 * kh, r, n),
                             lambda k: right(7 * kh * nh + cc), lambda k: key(2 * kh), start, finish, (live, live))

            def m2(m, v=v):
                v["c21"] = v["m2"] = m

            def m4(m, v=v, c=c):
                done(1, c, m + v["c21"])
                v["m4"] = m

            def m1(m, v=v):
                v["c11"], v["c22"] = m + v["m4"], m + v["c22"] if odd else m - v["m2"]

            def m3(m, v=v, c=c):
                done(1, nh + c, m + v["c22"])
                v["c12"] = m

            def m5(m, v=v, c=c):
                v["c11"], v["c12"] = v["c11"] - m, v["c12"] + m
                if not odd:
                    done(0, nh + c, v["c12"])

            def m7(m, v=v, c=c):
                v["c11"] = m
                if not odd:
                    done(0, c, m)

            get = lambda name, v=v: (lambda: v[name])
            put = lambda name, v=v: (lambda m: v.update({name: m}))
            e = held
            jobs += prod(1, none, m2, (1, 1))
            jobs += rest(1, c, get("c21"), put("c21"), 2)
            jobs += rest(1, nh + c, none, lambda m, v=v: v.update(c22=m - v["m2"]), 2)
            jobs += prod(3, none, m4, (2 + odd, 2 + e)) + prod(0, none, m1, (3 + e, 2 + e))
            jobs += prod(5, get("c22"), put("c22"), (2 + e, 2 + e)) + prod(2, none, m3, (3 + e, 2 + 2 * e))
            jobs += prod(4, none, m5, (3 + 2 * e, 2 + 2 * e)) + prod(6, get("c11"), m7, (2 + 2 * e, 2 * odd + 2 * e))
            jobs += rest(0, c, get("c11"), functools.partial(done, 0, c), 2 + 2 * e)
            jobs += rest(0, nh + c, get("c12"), functools.partial(done, 0, nh + c), 0)
        for c in range(2 * nh, nn):
            for half in range(2):
                jobs += chain(nk, functools.partial(plain_left, c, half),
                              lambda k: right(7 * kh * nh + odd * 2 * nh + k), key, none,
                              functools.partial(done, half, c))
        return jobs

    def weight_tasks(w_ref, col0, c_ref, nk, nn):
        kh, nh = nk // 2, nn // 2

        def combine(k, r, c):
            b = [w_ref[128 * (i * kh + k) + r:128 * (i * kh + k) + r + 16, _col(col0 + l * nh + c)].astype(F32)
                 for i in range(2) for l in range(2)]
            for term, val in enumerate(_right_terms(*b)):
                c_ref[_tile((term * kh + k) * nh + c, 64, r // 2, 8)] = _pack(val)
            return c_ref

        def copy(i, k, c):
            c_ref[_tile(7 * kh * nh + i, 64, 0, 64)] = _u32(w_ref[_col(k), _col(col0 + c)])
            return c_ref

        rest = [(k, c) for k in range(2 * kh, nk) for c in range(2 * nh)]
        rest += [(k, c) for c in range(2 * nh, nn) for k in range(nk)]
        return ([functools.partial(combine, k, r, c) for c in range(nh) for k in range(kh) for r in range(0, 128, 16)]
                + [functools.partial(copy, i, *kc) for i, kc in enumerate(rest)])

    def put_left(out, r, y, ks, n_terms):
        for k in ks:
            if k < KH:
                terms = _left_terms(y(0, k), y(0, KH + k), y(1, k), y(1, KH + k))
                for i in range(n_terms):
                    out[_tile(i * KH + k, RH, r // 2, 8)] = _pack(terms[i])
            else:
                for half in range(2):
                    out[_tile(9 * KH + half, RH, r // 2, 8)] = _pack(y(half, 2 * KH))

    def ln_tasks(src, stats, dst, row0, n_terms, lags):
        mean_s, rstd_s = stats
        order = [half * HB + r for r in range(0, HB, 16) for half in range(2)]

        def mean(r):
            v = jnp.sum(src(0)[r:r + 16, :].astype(F32), axis=-1, keepdims=True) * (1.0 / D)
            mean_s[r:r + 16, :] = jnp.broadcast_to(v, (16, 128))
            return mean_s if r == order[-1] or cur["pin_stats"] else None

        def rstd(r):
            cur["tl"].hold(mean_s, lags[0])
            c = src(1)[r:r + 16, :].astype(F32) - jnp.concatenate([dyn(mean_s)[r:r + 16, :]] * ND, axis=1)
            v = jnp.sum(c * c, axis=-1, keepdims=True) * (1.0 / D)
            rstd_s[r:r + 16, :] = jnp.broadcast_to(lax.rsqrt(v + EPS), (16, 128))
            return rstd_s if r == order[-1] or cur["pin_stats"] else None

        def norm(r, ks):
            cur["tl"].hold(rstd_s, lags[1])

            def y(half, c):
                rows = slice(half * HB + r, half * HB + r + 16)
                return (src(2)[rows, _col(c)].astype(F32) - dyn(mean_s, zero)[rows, :]) * dyn(rstd_s)[rows, :]

            put_left(dst.at[_at(row0, XR, 8)], r, y, ks, n_terms)
            return dst

        return ([functools.partial(mean, r) for r in order], [functools.partial(rstd, r) for r in order],
                [functools.partial(norm, r, ks) for r in range(0, HB, 16) for ks in cur["norm"]])

    def ln1_tasks(j, times):
        sweeps = ln_tasks(lambda i: dyn(x_s, j * TB + i * zero, TB, 16), ln1_s, xn_s, j % 2 * XR, 9, cur["hold_ln1"])
        return list(zip(sweeps, times))

    def ln2_tasks(j):
        mean, rstd, norm = ln_tasks(lambda i: dyn(h_s, j * TB + i * zero, TB), ln2_s, hn_s, 0, 7, cur["hold_ln2"])
        return mean + [None] + rstd + [g for f in norm for g in (f, None)][:-1]

    def ln1_now(j):
        for r in range(0, HB, 16):
            ys = []
            for half in range(2):
                x = x_s[j * TB + half * HB + r:j * TB + half * HB + r + 16, :].astype(F32)
                c = x - jnp.sum(x, axis=-1, keepdims=True) * (1.0 / D)
                ys.append(c * lax.rsqrt(jnp.sum(c * c, axis=-1, keepdims=True) * (1.0 / D) + EPS))
            put_left(xn_s.at[pl.ds(j * XR, XR)], r, lambda half, c: ys[half][:, _col(c)], (KH, *range(KH)), 9)

    def qkv_jobs(j, i, done):
        if isinstance(j, int) and j < 2 and i == 0:
            def lhs(c, half, k, r, n):
                t = _QUADRANT[half][k // KH] * KH + k % KH if k < 2 * KH else 9 * KH + half
                return dyn(xn_s, j * XR + c * zero, XR)[_tile(t, RH, r // 2, n // 2)]
            return [job for c in range(ND) for half in range(2) for job in chain(
                ND, functools.partial(lhs, c, half), lambda k, c=c: wqkv_s[_col(k), _col(c)], lambda k: (),
                lambda: None, functools.partial(done, half, c))]
        return gemm_jobs(xn_s, j % 2 * XR, XR, i * ND, cqkv_s[i], ND, ND, done, lambda k: (("w", i),))

    def q_jobs(j):
        buf = q_s[j % 2 if isinstance(j, int) else 0]

        def done(half, c, v):
            buf[half * RH:(half + 1) * RH, _col(c)] = _pack(v * QSCALE)

        def flip(c):
            qt_s[64 * c:64 * c + 64, _at(j * TB, TB, TB)] = _u32(_bf(dyn(buf)[:, _col(c)]).T)
            return qt_s
        return qkv_jobs(j, 0, done), [functools.partial(flip, c) for c in range(ND)]

    def k_jobs(j):
        def done(half, c, v):
            k_s[_at(j * RB + half * RH + 48, RH, 8), _col(c)] = _pack(v)
        return qkv_jobs(j, 1, done)

    def v_jobs(j):
        buf = v_s[j % 2 if isinstance(j, int) else 0]
        sub = _iota((8, TB), 0)

        def done(half, c, v):
            buf[half * RH:(half + 1) * RH, _col(c)] = _pack(v)

        def flip(c):
            vp_s[64 * c:64 * c + 64, :] = _u32(_bf(dyn(buf)[:, _col(c)]).T)
            return vp_s

        def widen(c, i0):
            vt = _bf(dyn(vp_s)[64 * c + 4 * i0:64 * c + 4 * i0 + 32, :]).astype(F32)
            cols = _at(j * TB, TB, TB)
            for i in range(8):
                pair, m = divmod(16 * c + i0 + i, 5)
                t, r = vt[8 * i:8 * i + 8], 48 * pair + 8 * (m if m <= 2 else m + 1)
                if m == 2:
                    vt_s[r:r + 8, cols] = jnp.where(sub < 4, t, 1.0)
                    vt_s[r + 8:r + 16, cols] = jnp.where(sub < 4, 1.0, t)
                else:
                    vt_s[r:r + 8, cols] = t
            return vt_s

        tasks = [functools.partial(flip, c) for c in range(ND)]
        return qkv_jobs(j, 2, done), tasks + [functools.partial(widen, c, i) for c in range(ND) for i in (0, 8)]

    def skew_tasks(j):
        lane = _iota((8, 128), 1)
        cuts, lag = cur["skew_cuts"], cur["hold_skew"]

        def task(r):
            cur["tl"].hold(k_s, lag)
            src, dst = dyn(k_s, j * RB + r, 8 + 48), ks_s.at[_at(j * RB, RB, 8)]
            prev = None
            for t in range(ND):
                head = ((128 * t + lane) * 3277) >> 16
                ks = [src[16 * s:16 * s + 8, _col(t)] for s in range(4)]
                odd = (head & 1) == 1
                e = [[jnp.where(odd, ks[2 * hi + 1], ks[2 * hi]) for hi in range(2)],
                     [jnp.where(odd, ks[2 * hi], ks[2 * hi + 1]) for hi in range(2)]]
                new = [jnp.where(((head - u % 2) & 2) == 2, e[u % 2][1 - u // 2], e[u % 2][u // 2]) for u in range(4)]
                for g in range(NG):
                    t0, t1 = 80 * g // 128, (80 * g + 79) // 128
                    if t1 == t:
                        for u in range(4):
                            v = new[u] if t0 == t1 else jnp.where(lane >= 80 * g % 128, prev[u], new[u])
                            dst[r:r + 8, _col(u * NG + g)] = v
                prev = new
                if t in cuts:
                    yield ks_s

        gens = [task(r) for r in range(0, RB, 8)]
        return [functools.partial(next, gen) for gen in gens for _ in cuts]

    def wo_jobs(j):
        def done(half, c, v):
            rows = _at(j * TB + half * HB, HB, HB)
            h_s[rows, _col(c)] = x_s[rows, _col(c)].astype(F32) + v
        return gemm_jobs(o_s, 0, None, 0, co_s, ND, ND, done, lambda k: (("o", k),))

    def ffn1_jobs(buf):
        held = {}

        def done(half, c, v):
            held[half, c] = jnp.maximum(v, 0.0)
            k = c % FH
            if half == 1 and (1, k) in held and (1, FH + k) in held:
                a21, a22 = held[1, k], held[1, FH + k]
                for i, val in ((1, a21 + a22), (3, a22), (8, a21)):
                    buf[_tile(i * FH + k, RH, 0, RH)] = _pack(val)
            elif (0, k) in held and (0, FH + k) in held:
                terms = _left_terms(held[0, k], held[0, FH + k], held[1, k], held[1, FH + k])
                for i in (0, 2, 4, 5, 6, 7):
                    buf[_tile(i * FH + k, RH, 0, RH)] = _pack(terms[i])
        return gemm_jobs(hn_s, 0, None, 0, c1_s, ND, NF, done, lambda k: ("hn",), held=1)

    def ffn2_jobs(j, buf):
        def done(half, c, v):
            rows = _at(j * TB + half * HB, HB, HB)
            out_s[rows, _col(c)] = (h_s[rows, _col(c)] + v).astype(BF)
        return gemm_jobs(buf, 0, None, 0, c2_s, NF, ND, done)

    def run_round(tl, jobs):
        if len(jobs) >= 4:
            tl.round(jobs[:4], HB)
            del jobs[:4]
            return
        assert len(jobs) == 2
        n, res = HB // 2, [[], []]
        tl.round([(lambda r, m, i=i, job=job: job[0](i * n + r, m), job[1], out.append, job[3])
                  for job, out in zip(jobs, res) for i in range(2)], n)
        for job, out in zip(jobs, res):
            job[2](jnp.concatenate(out, axis=0))
        del jobs[:]

    lane32, lane16, lane8, sub8 = _iota((32, 128), 1), _iota((16, 128), 1), _iota((8, 128), 1), _iota((8, 128), 0)
    causal = _iota((32, 128), 0) <= (lane32 & 31)
    first_chunk = {1: 5, 2: 1, 3: 0}

    def scores(tl, qb, g, nk, slot):
        c_lo = first_chunk[nk]
        keys = dyn(ks_s, qb * 64 - 80 + 16 * c_lo, 16 * (9 - c_lo))

        def lhs(u, r, n):
            return keys[r // 2:(r + n) // 2, _col(u * NG + g)]

        def rhs(u):
            tiles = [jnp.zeros((8, 128), U32)] * 8
            for i in range(5):
                head = sum((16 * i + 2 * sub8 >= DH * a).astype(I32) for a in range(1, 4))
                q = qt_s[40 * g + 8 * i:40 * g + 8 * i + 8, _at(qb * 128, 128, 128)]
                tiles[(5 * g + i) % 8] = jnp.where(((head - (lane8 >> 5)) & 3) == u, q, jnp.uint32(0))
            return _bf(jnp.concatenate(tiles, axis=0))

        def done(u, s):
            ch = {c: s[32 * (c - c_lo):32 * (c - c_lo + 1)] for c in range(c_lo, 9)}
            if nk == 3:
                ch[8] = jnp.where(causal, ch[8], ch.pop(0))
            else:
                ch[8] = jnp.where(causal, ch[8], -jnp.inf)
                for c in range(c_lo, c_lo + 3):
                    ch[c] = jnp.where((lane32 >> 5) >= c_lo + 3 - c, ch[c], -jnp.inf)
            mx = None
            for c in sorted(ch):
                for r in range(0, 32, 8):
                    mx = ch[c][r:r + 8] if mx is None else jnp.maximum(mx, ch[c][r:r + 8])
                s_s[slot][32 * c - 32:32 * c, _col(u)] = ch[c]
            s_s[slot][256:264, _col(u)] = jnp.broadcast_to(jnp.max(mx, axis=0, keepdims=True), (8, 128))

        tl.round([(functools.partial(lhs, u), functools.partial(rhs, u), functools.partial(done, u), ())
                  for u in range(4)], 32 * (9 - c_lo))

    def exp_tasks(nk, slot):
        def task(u, c):
            src = dyn(s_s[slot])
            mx = jnp.concatenate([src[256:264, _col(u)]] * 4, axis=0)
            p = jnp.exp2(src[32 * c - 32:32 * c, _col(u)] - mx)
            if c == 8 and nk == 3:
                p_s[slot][0:16, _col(u)] = _pack(jnp.where(causal, 0.0, p))
                p = jnp.where(causal, p, 0.0)
            p_s[slot][16 * c:16 * c + 16, _col(u)] = _pack(p)
            return p_s[slot]
        return [functools.partial(task, u, c) for c in (8, *range(max(first_chunk[nk], 1), 8)) for u in range(4)]

    def values(tl, qb, g, nk, slot):
        tl.need({("p", slot)})

        def prob(u, c):
            if first_chunk[nk] <= c < 9:
                return dyn(p_s[slot])[16 * c:16 * c + 16, _col(u % 4)]
            return jnp.zeros((16, 128), U32)

        def shifted(a, c):
            if not first_chunk[nk] <= c < 10:
                return jnp.zeros((16, 128), U32)
            same, lower = prob(a, c), prob(a - 1, c - 1)
            return jnp.where((lane16 & 32) != 0, lower, same)

        o = [None] * 4
        for kt in range(3 - nk, 3):
            for a in range(4):
                p = [jnp.where((lane16 & 64) != 0, shifted(a - 2, c - 2), shifted(a, c))
                     for c in range(4 * kt, 4 * kt + 4)]
                v = vt_s[24 * (4 * g + a):24 * (4 * g + a + 1), _at((qb - 2 + kt) * 128, 128, 128)]
                r = _mm(v, _bf(jnp.concatenate(p, axis=0)))
                o[a] = r if o[a] is None else r + o[a]
        for a in (0, 2):
            e, f = o[a], o[a + 1]
            total = jnp.where(sub8 < 4, f[0:8], e[16:24])
            inv = pltpu.reciprocal(total, approx=True)
            inv = inv * (2.0 - total * inv)
            e, f = e * inv[4:5], f * inv[0:1]
            for i, v in enumerate([e[0:8], e[8:16], jnp.where(sub8 < 4, e[16:24], f[0:8]), f[8:16], f[16:24]]):
                t, row = divmod(80 * g + 20 * a + 8 * i, 128)
                ot_s[t][row:row + 8, _col(slot)] = v

    def o_tasks(k):
        def quad(half, l):
            return dyn(ot_s[k + l * KH])[:, _col(half)]

        def task(i):
            if k < KH:
                v, t = _left_terms(quad(0, 0), quad(0, 1), quad(1, 0), quad(1, 1))[i], i * KH + k
            else:
                v, t = quad(i, 0), 9 * KH + i
            o_s[_tile(t, RH, 0, RH)] = _u32(v.astype(BF).T)
            return o_s
        return [functools.partial(task, i) for i in range(9 if k < KH else 2)]

    def step(segments, extra=(), j=None, attn=False, prev_attn=False, first_exp=None):
        tl = cur["tl"] = _Timeline(pin, cur["chunk"], cur["turns"])
        jobs, marks, o_ready = [], [], []
        for js, *after in segments:
            jobs += js
            if after:
                marks.append((len(jobs), *after))
        total, n_steps = len(jobs), 2 * NG

        def nk(s):
            return 1 + s % 2 if isinstance(j, int) and j + s // n_steps == 0 else 3

        def live(s):
            return attn if s >= 0 else prev_attn

        span = total * HB / 4 + (sum(32 * (9 - first_chunk[nk(s)]) for s in range(n_steps)) if attn else 0)
        for tasks, (t0, t1), *key in extra:
            tl.spread(t0 * span, t1 * span, tasks, *key)
        if prev_attn:
            tl.spread(cur["o_first"], cur["o_first"] + cur["o_span"], o_tasks(KH - 1), ("o", KH - 1))
        o_free = not any(("o", 0) in job[3] for job in jobs)
        rounds = (total + 3) // 4
        cuts = _choose_cuts(jobs, n_steps, cur["even"]) if attn else [0, 4, 6, rounds] if prev_attn else [0, rounds]
        for s in range(len(cuts) - 1):
            n = cuts[s + 1] - cuts[s]
            if live(s - 1):
                t0 = tl.t + (cur["exp"][0] if s else first_exp or cur["chunk"])
                t1 = tl.t + sum(HB if len(jobs) - 4 * i >= 4 else HB // 2 for i in range(n)) + attn * cur["exp"][1]
                tl.spread(t0, max(t0, t1), exp_tasks(nk(s - 1), (s - 1) % 2), ("p", (s - 1) % 2))
            for _ in range(n):
                assert not (prev_attn and s < 2 and any(("o", 2 * KH) in job[3] for job in jobs[:4]))
                before = total - len(jobs)
                run_round(tl, jobs)
                for end, tasks, length, *key in marks:
                    if before < end <= total - len(jobs):
                        tl.spread(tl.t + cur["after"], tl.t + cur["after"] + length, tasks, *key)
                        o_free = o_free or key == ["hn"]
            if live(s - 2):
                values(tl, 2 * j + s % 2 - 2 * (s < 2), (s - 2) // 2 % NG, nk(s - 2), s % 2)
                if s == 1:
                    tl.spread(tl.t + cur["o_after"], tl.t + cur["o_after"] + 64, o_tasks(2 * KH), ("o", 2 * KH))
                o_ready += [k for k in range(KH - 1) if s - 2 == 2 * ((128 * (KH + k) + 127) // 80) + 1]
            while o_ready and o_free:
                t0 = tl.t + cur["o_after"]
                tl.spread(t0, t0 + cur["o_span"], o_tasks(o_ready.pop(0)))
            if attn:
                scores(tl, 2 * j + s % 2, s // 2, nk(s), s % 2)
        tl.run(float("inf"))

    def send(cp):
        def task():
            cp.start()
            dyn(out_s, multiple=16)[S:, _col(0)] = jnp.zeros((2 * SPARE, 128), BF)
            return out_s
        return [task], 0

    (q0, q0_flip), (q1, q1_flip), (v1, v1_flip), k1 = q_jobs(0), q_jobs(1), v_jobs(1), k_jobs(1)
    qkv_weights = [weight_tasks(wqkv_s, i * ND, cqkv_s[i], ND, ND) for i in range(3)]
    late_weights = (weight_tasks(wo_s, 0, co_s, ND, ND) + weight_tasks(w1_s, 0, c1_s, ND, NF)
                    + weight_tasks(w2_s, 0, c2_s, NF, ND))
    n_head, n_next = ND * 2 * head // 4 * 4, 16

    def start0(part):
        pace("start0")
        step([(q0[:n_head] if part == 0 else q0[n_head:] + q1[:n_next],)])

    def start1():
        pace("start1")
        t = cur["t"]
        step([(q1[n_next:] + k_jobs(0) + k1[:2],)],
             [(qkv_weights[1], t[0], ("w", 1)), (q0_flip, t[1]), (qkv_weights[0], t[2]), (q1_flip, t[3])])

    def start2():
        pace("start2")
        t = cur["t"]
        step([(k1[2:],), (*v_jobs(0), cur["v_span"]), (v1,)],
             [(qkv_weights[2], t[0], ("w", 2)), *ln1_tasks(2, t[1:4]), (skew_tasks(0), t[4])])

    def proj(j):
        pace("proj")
        t = cur["t"]
        step([(*q_jobs(j), cur["q_span"]), (*v_jobs(j), cur["v_span"]), (k_jobs(j),)],
             [*ln1_tasks(j + 1, t[:3]), (skew_tasks(j - 1), t[3])])

    def attn0():
        pace("attn0")
        j, t, cut = NB - 2, cur["t"], int(len(late_weights) * cur["share"])
        step([(*q_jobs(j), cur["q_span"]), (*v_jobs(j), cur["v_span"]), (k_jobs(j),)],
             [(late_weights[:cut], t[0]), (v1_flip[:ND], t[1]), (v1_flip[ND:], t[2]), (skew_tasks(j - 1), t[3]),
              *ln1_tasks(j + 1, t[4:])], j=0, attn=True)

    def attn1():
        pace("attn1")
        j, t, cut = NB - 1, cur["t"], int(len(late_weights) * _PACES["attn0"]["share"])
        ready = len(late_weights) - len(weight_tasks(w2_s, 0, c2_s, NF, ND))
        mid = t[1][0] + (t[1][1] - t[1][0]) * (ready - cut) / (len(late_weights) - cut - 1)
        step([(*q_jobs(j), cur["q_span"]), (wo_jobs(0), ln2_tasks(0), cur["ln_span"], "hn"),
              (k_jobs(j), skew_tasks(j), cur["skew_span"]), (*v_jobs(j), cur["v_span"]), (ffn1_jobs(a_s[0]),)],
             [(skew_tasks(j - 1), t[0]), (late_weights[cut:ready] + [None], (t[1][0], mid), "hn"),
              (late_weights[ready:], (mid, t[1][1]))],
             j=1, attn=True, prev_attn=True, first_exp=cur["exp"][0])

    def main(j):
        pace("main")
        f2 = ffn2_jobs(j - 2, a_s[0])
        step([(f2[:cur["cut"]],), (wo_jobs(j - 1), ln2_tasks(j - 1), cur["ln_span"], "hn"),
              (f2[cur["cut"]:], [lambda: out_cp(j - 2).start()], 0), (ffn1_jobs(a_s[0]),)],
             j=j, attn=True, prev_attn=True)

    def finish():
        pace("finish")
        f2, last, (c0, c1) = ffn2_jobs(NB - 2, a_s[0]), ffn2_jobs(NB - 1, a_s[1]), cur["cut"]
        n = 7 * FH * KH
        step([(f2[:c0],), (wo_jobs(NB - 1), ln2_tasks(NB - 1), cur["ln_span"], "hn"),
              (f2[c0:c1] + ffn1_jobs(a_s[1]),), (f2[c1:], *send(out_cp(NB - 2))),
              (last[:n], *send(out_cp(NB - 1, 0, 2 * KH))), (last[n:],)], j=NB, prev_attn=True)

    def loop(lo, hi, body):
        lax.fori_loop(0, hi - lo, lambda i, carry: body(lo + zero + i), None)

    x_cp(0).wait()
    ln1_now(0)
    wk_cp.start()
    wq_head.wait()
    start0(0)
    x_cp(1).wait()
    ln1_now(1)
    wq_rest.wait()
    start0(1)
    wv_cp.start()
    x_cp(2).start()
    wk_cp.wait()
    start1()
    for i in range(3, NB):
        x_cp(i).start()
    wv_cp.wait()
    x_cp(2).wait()
    start2()
    for cp in late_cps:
        cp.start()
    for i in range(3, NB):
        x_cp(i).wait()
    loop(2, NB - 2, proj)
    for cp in late_cps:
        cp.wait()
    attn0()
    attn1()
    loop(2, NB, main)
    finish()
    out_cp(NB - 1, 2 * KH, ND).start()
    for i in range(NB - 1):
        out_cp(i).wait()
    out_cp(NB - 1, 0, 2 * KH).wait()
    out_cp(NB - 1, 2 * KH, ND).wait()


def _layer(x, wqkv, wo, w1, w2):
    (S, D), FF = x.shape, w1.shape[1]
    nd, nf = D // 128, FF // 128
    vmem = pltpu.VMEM

    def tiled(count, rows, dtype=U32, blocks=1):
        return vmem((blocks * -(-count // 4) * rows + SPARE, 512), dtype)

    def right(nk, nn):
        return tiled(7 * (nk // 2) * (nn // 2) + nk * nn - nk // 2 * 2 * (nn // 2 * 2), 64)

    left = 9 * (nd // 2) + 2
    stats = [vmem((TB + 32, 128), F32)] * 2
    hbm = pl.BlockSpec(memory_space=pl.ANY)
    return pl.pallas_call(
        _kernel,
        in_specs=[hbm] * 5,
        out_specs=hbm,
        out_shape=jax.ShapeDtypeStruct((S, D), x.dtype),
        scratch_shapes=[
            vmem((S, D), BF), vmem((D, 3 * D), BF), vmem((D, D), BF), vmem((D, FF), BF), vmem((FF, D), BF),
            [right(nd, nd)] * 3, right(nd, nd), right(nd, nf), right(nf, nd), stats, stats,
            tiled(left, RH, blocks=2), [vmem((RB, D), U32)] * 2, [vmem((RB, D), U32)] * 2,
            vmem((D // 2 + 16, TB), U32), vmem((D // 2 + SPARE, S), U32), vmem((S // 2 + 64, D), U32),
            vmem((S // 2 + SPARE, 128 * H), U32), vmem((24 * H + SPARE, S), F32),
            [vmem((264, 512), F32)] * 2, [vmem((144 + SPARE, 512), U32)] * 2, [vmem((128, TB), F32)] * nd,
            tiled(left, RH), vmem((S, D), F32), tiled(left, RH), [tiled(9 * (nf // 2), RH)] * 2,
            vmem((S + 2 * SPARE, D), BF),
            pltpu.SemaphoreType.DMA((7,)), pltpu.SemaphoreType.DMA((S // TB,)), pltpu.SemaphoreType.DMA((S // TB + 1,)),
        ],
        compiler_params=pltpu.CompilerParams(vmem_limit_bytes=100 << 20),
        name="fused_layer",
    )(x, wqkv, wo, w1, w2)


@jax.jit
def pallas_sequential_preLN__sliding_block__dense_activation_relu__prompt_kernel(
    A_x: jax.Array,
    A_wqkv: jax.Array,
    A_wo: jax.Array,
    B_x: jax.Array,
    B_w1: jax.Array,
    B_w2: jax.Array,
):
    del B_x
    return _layer(A_x.reshape(A_x.shape[-2:]), A_wqkv, A_wo, B_w1, B_w2).reshape(A_x.shape)
```

```python
import functools
import heapq

import jax
import jax.numpy as jnp
import numpy as np
from jax import lax
from jax.experimental import pallas as pl
from jax.experimental.pallas import tpu as pltpu

BF, F32, U32, I32 = jnp.bfloat16, jnp.float32, jnp.uint32, jnp.int32
H, DH = 32, 20
NG = H // 4
TB = 256
HB = TB // 2
RB, RH = TB // 2, HB // 2
SPARE = 8
EPS = 1e-5
QSCALE = float(DH ** -0.5 * np.log2(np.e))

_PACE = dict(chunk=16, turns=1, even=1.5, after=300, exp=(192, 96), o_first=288, o_after=600, o_span=1000,
             q_span=900, v_span=1000, pin_stats=True, norm=((0, 1, 2),), hold_ln1=(512, 224), hold_ln2=(512, 256),
             hold_skew=224, skew_cuts=(2, 4))
_PACES = dict(
    start0=dict(),
    start1=dict(chunk=32, t=((0.02, 0.4), (0.1, 0.4), (0.5, 0.95), (0.6, 0.9))),
    start2=dict(chunk=32, cut=18, v_last=500, v_span=800, pin_stats=False, after=400, norm=((0,), (1, 2)),
                skew_cuts=(1, 2, 3, 4), t=((0.01, 0.09), (0.12, 0.2), (0.24, 0.42), (0.5, 0.8), (0.2, 0.6))),
    proj=dict(chunk=32, after=400, q_span=600, v_span=800, pin_stats=False, hold_ln1=(400, 224),
              norm=((0,), (1, 2)), skew_cuts=(1, 2, 3, 4), t=((0.04, 0.14), (0.18, 0.38), (0.5, 0.8), (0.15, 0.66))),
    attn0=dict(turns=2, even=5, after=400, o_span=1500, pin_stats=False, exp=(224, 96), q_span=1200, v_span=1200, norm=((0,), (1,), (2,)), share=0.33,
               t=((0.02, 0.97), (0.3, 0.64), (0.03, 0.08), (0.12, 0.3), (0.33, 0.6))),
    attn1=dict(turns=2, even=5, after=400, q_span=2400, v_span=3000, skew_cuts=(1, 2, 3, 4), ln_span=2400,
               skew_span=4000, t=((0.01, 0.33), (0.02, 0.97))),
    main=dict(cut=44, ln_span=2200),
    finish=dict(cut=(40, 100), ln_span=1500),
)


def _mm(a, b):
    return lax.dot_general(a, b, (((1,), (0,)), ((), ())), preferred_element_type=F32)


def _iota(shape, d):
    return lax.broadcasted_iota(I32, shape, d)


def _at(start, n, multiple):
    return pl.ds(start if isinstance(start, int) else pl.multiple_of(start, multiple), n)


def _u32(x):
    return pltpu.bitcast(x, U32)


def _bf(x):
    return pltpu.bitcast(x, BF)


def _pack(x):
    return _u32(x.astype(BF))


def _col(c, n=1):
    return slice(128 * c, 128 * (c + n))


def _tile(i, rows, r, n):
    return slice(i // 4 * rows + r, i // 4 * rows + r + n), _col(i % 4)


def _left_terms(a11, a12, a21, a22):
    return [a11 + a22, a21 + a22, a11, a22, a11 + a12, a21 - a11, a12 - a22, a12, a21]


def _right_terms(b11, b12, b21, b22):
    return [b11 + b22, b11, b12 - b22, b21 - b11, b22, b11 + b12, b21 + b22]


_QUADRANT = ((2, 7), (8, 3))


def _choose_cuts(jobs, n, even):
    rounds = (len(jobs) + 3) // 4
    open_at = [0] + [jobs[min(4 * r, len(jobs)) - 1][4] for r in range(1, rounds + 1)]
    best = {0: (0.0, [0])}
    for _ in range(n):
        best = {r: min((cost + open_at[r] + even * (r - p - rounds / n) ** 2, path + [r])
                       for p, (cost, path) in best.items() if p < r)
                for r in range(min(best) + 1, rounds + 1)}
    return best[rounds][1]


class _Timeline:
    def __init__(self, pin, chunk, turns):
        self.pin, self.chunk, self.turns = pin, chunk, turns
        self.t = self.now = self.count = self.turn = 0
        self.queue, self.stored, self.results = [], {}, []

    def spread(self, t0, t1, tasks, key=None):
        for i, task in enumerate(tasks):
            if task is not None:
                heapq.heappush(self.queue, (t0 + (t1 - t0) * i / max(len(tasks) - 1, 1), self.count, task, key))
                self.count += 1

    def run(self, t):
        self.now = t
        while self.queue and self.queue[0][0] <= t:
            ref = heapq.heappop(self.queue)[2]()
            if ref is not None:
                self.stored[id(ref)] = ref

    def need(self, keys):
        due = sorted(e for e in self.queue if e[3] in keys)
        self.queue = [e for e in self.queue if e[3] not in keys]
        heapq.heapify(self.queue)
        for e in due:
            e[2]()

    def hold(self, ref, lag):
        old = [v for t, v in self.results if t <= self.now - lag]
        if old:
            ref[ref.shape[0] - SPARE:, _col(0)] = old[-1] if ref.dtype == F32 else _u32(old[-1])

    def round(self, jobs, rows):
        parts = [[] for _ in jobs]
        self.need({k for job in jobs for k in job[3]})
        for r in range(0, rows, self.chunk):
            self.run(self.t + r)
            for p, job in zip(parts, jobs):
                p.append(job[0](r, self.chunk))
            for ref in self.stored.values():
                self.turn = (self.turn + 1) % self.turns
                parts[self.turn][-1] = self.pin(parts[self.turn][-1], ref)
            self.stored = {}
        for p, job in zip(parts, jobs):
            res = _mm(_bf(jnp.concatenate(p, axis=0)), job[1]())
            out = job[2](res)
        out = res if out is None else out
        self.results += [(self.t + r, out[r:r + SPARE]) for r in range(0, rows, self.chunk)]
        self.t += rows


def _kernel(x_hbm, wqkv_hbm, wo_hbm, w1_hbm, w2_hbm, out_hbm,
            x_s, wqkv_s, wo_s, w1_s, w2_s, cqkv_s, co_s, c1_s, c2_s, ln1_s, ln2_s, xn_s, q_s, v_s, vp_s,
            qt_s, k_s, ks_s, vt_s, s_s, p_s, ot_s, o_s, h_s, hn_s, a_s, out_s, sem_w, sem_x, sem_out):
    (S, D), FF = x_hbm.shape, w1_hbm.shape[1]
    NB, ND, NF = S // TB, D // 128, FF // 128
    KH, FH = ND // 2, NF // 2
    XR = o_s.shape[0] - SPARE
    cur = {}

    def pace(name):
        cur.update(_PACE, **_PACES[name])

    def x_cp(i):
        return pltpu.make_async_copy(x_hbm.at[pl.ds(i * TB, TB)], x_s.at[pl.ds(i * TB, TB)], sem_x.at[i])

    def out_cp(i, c0=0, c1=ND):
        at = (_at(i * TB, TB, TB), pl.ds(128 * c0, 128 * (c1 - c0)))
        return pltpu.make_async_copy(out_s.at[at], out_hbm.at[at], sem_out.at[i + (c0 > 0)])

    head = 3
    wq_head, wq_rest, wk_cp, wv_cp = [
        pltpu.make_async_copy(wqkv_hbm.at[:, pl.ds(c0, c1 - c0)], wqkv_s.at[:, pl.ds(c0, c1 - c0)], sem_w.at[i])
        for i, (c0, c1) in enumerate(((0, 128 * head), (128 * head, D), (D, 2 * D), (2 * D, 3 * D)))]
    late_cps = [pltpu.make_async_copy(src, dst, sem_w.at[4 + i])
                for i, (src, dst) in enumerate(((wo_hbm, wo_s), (w1_hbm, w1_s), (w2_hbm, w2_s)))]
    for cp in (x_cp(0), wq_head, x_cp(1), wq_rest):
        cp.start()

    k_s[0:48, :] = jnp.zeros((48, D), U32)
    for ref in (*cqkv_s, co_s, c1_s, c2_s, *ln1_s, *ln2_s, xn_s, vp_s, qt_s, ks_s, vt_s, *p_s, o_s, hn_s):
        ref[ref.shape[0] - SPARE:, _col(0)] = jnp.zeros((SPARE, 128), ref.dtype)

    zero = lax.fori_loop(0, 2, lambda i, c: i * (i - 1) * (2 * i - 1) * 128, jnp.int32(0))
    keep = _iota((8, 128), 0) >= zero

    def dyn(ref, row=0, n=None, multiple=8):
        return ref.at[_at(zero + row, n or ref.shape[0], multiple)]

    def pin(v, ref):
        n = 2 * SPARE if ref.dtype == BF else SPARE
        w = dyn(ref, multiple=n)[ref.shape[0] - n:, _col(0)]
        first = jnp.where(keep, v[0:8], w if w.dtype == U32 else _u32(w))
        return jnp.concatenate([first, v[8:]], axis=0) if v.shape[0] > 8 else first

    def chain(n, lhs, rhs, key, start, finish, live=(1, 0)):
        acc = []

        def done(r):
            prev = acc[-1] if acc else start()
            acc.append(r if prev is None else r + prev)
            if len(acc) == n:
                finish(acc[-1])
            return acc[-1]
        return [(functools.partial(lhs, k), functools.partial(rhs, k), done, key(k), live[k == n - 1])
                for k in range(n)]

    def gemm_jobs(a_ref, row0, rows, tag, c_ref, nk, nn, done, key=lambda k: (), held=0):
        kh, nh, odd = nk // 2, nn // 2, nk % 2
        none = lambda: None

        def left(c, term, k, r, n):
            return dyn(a_ref, row0 + (tag + c) * zero, rows)[_tile(term * kh + k, RH, r // 2, n // 2)]

        def plain_left(c, half, k, r, n):
            if k < 2 * kh:
                return left(c, _QUADRANT[half][k // kh], k % kh, r, n)
            return left(c, 9, half, r, n)

        def right(i):
            return _bf(dyn(c_ref)[_tile(i, 64, 0, 64)])

        jobs = []
        for c in range(nh):
            v = {}

            def prod(term, start, finish, live, c=c):
                return chain(kh, functools.partial(left, c, term), lambda k: right((term * kh + k) * nh + c),
                             lambda k: key(k) + key(kh + k), start, finish, live)

            def rest(half, cc, start, finish, live):
                return chain(odd, lambda k, r, n: plain_left(cc, half, 2 * kh, r, n),
                             lambda k: right(7 * kh * nh + cc), lambda k: key(2 * kh), start, finish, (live, live))

            def m2(m, v=v):
                v["c21"] = v["m2"] = m

            def m4(m, v=v, c=c):
                done(1, c, m + v["c21"])
                v["m4"] = m

            def m1(m, v=v):
                v["c11"], v["c22"] = m + v["m4"], m + v["c22"] if odd else m - v["m2"]

            def m3(m, v=v, c=c):
                done(1, nh + c, m + v["c22"])
                v["c12"] = m

            def m5(m, v=v, c=c):
                v["c11"], v["c12"] = v["c11"] - m, v["c12"] + m
                if not odd:
                    done(0, nh + c, v["c12"])

            def m7(m, v=v, c=c):
                v["c11"] = m
                if not odd:
                    done(0, c, m)

            get = lambda name, v=v: (lambda: v[name])
            put = lambda name, v=v: (lambda m: v.update({name: m}))
            e = held
            jobs += prod(1, none, m2, (1, 1))
            jobs += rest(1, c, get("c21"), put("c21"), 2)
            jobs += rest(1, nh + c, none, lambda m, v=v: v.update(c22=m - v["m2"]), 2)
            jobs += prod(3, none, m4, (2 + odd, 2 + e)) + prod(0, none, m1, (3 + e, 2 + e))
            jobs += prod(5, get("c22"), put("c22"), (2 + e, 2 + e)) + prod(2, none, m3, (3 + e, 2 + 2 * e))
            jobs += prod(4, none, m5, (3 + 2 * e, 2 + 2 * e)) + prod(6, get("c11"), m7, (2 + 2 * e, 2 * odd + 2 * e))
            jobs += rest(0, c, get("c11"), functools.partial(done, 0, c), 2 + 2 * e)
            jobs += rest(0, nh + c, get("c12"), functools.partial(done, 0, nh + c), 0)
        for c in range(2 * nh, nn):
            for half in range(2):
                jobs += chain(nk, functools.partial(plain_left, c, half),
                              lambda k: right(7 * kh * nh + odd * 2 * nh + k), key, none,
                              functools.partial(done, half, c))
        return jobs

    def weight_tasks(w_ref, col0, c_ref, nk, nn):
        kh, nh = nk // 2, nn // 2

        def combine(k, r, c):
            b = [w_ref[128 * (i * kh + k) + r:128 * (i * kh + k) + r + 16, _col(col0 + l * nh + c)]
                 for i in range(2) for l in range(2)]
            for term, val in enumerate(_right_terms(*[t.astype(F32) for t in b])):
                val = _u32(b[0]) if term == 1 else _u32(b[3]) if term == 4 else _pack(val)
                c_ref[_tile((term * kh + k) * nh + c, 64, r // 2, 8)] = val
            return c_ref

        def copy(i, k, c):
            c_ref[_tile(7 * kh * nh + i, 64, 0, 64)] = _u32(w_ref[_col(k), _col(col0 + c)])
            return c_ref

        rest = [(k, c) for k in range(2 * kh, nk) for c in range(2 * nh)]
        rest += [(k, c) for c in range(2 * nh, nn) for k in range(nk)]
        return ([functools.partial(combine, k, r, c) for c in range(nh) for k in range(kh) for r in range(0, 128, 16)]
                + [functools.partial(copy, i, *kc) for i, kc in enumerate(rest)])

    def put_left(out, r, y, ks, n_terms):
        for k in ks:
            if k < KH:
                terms = _left_terms(y(0, k), y(0, KH + k), y(1, k), y(1, KH + k))
                for i in range(n_terms):
                    out[_tile(i * KH + k, RH, r // 2, 8)] = _pack(terms[i])
            else:
                for half in range(2):
                    out[_tile(9 * KH + half, RH, r // 2, 8)] = _pack(y(half, 2 * KH))

    def ln_tasks(src, stats, dst, row0, n_terms, lags):
        mean_s, rstd_s = stats
        order = [half * HB + r for r in range(0, HB, 16) for half in range(2)]

        def mean(r):
            v = jnp.sum(src(0)[r:r + 16, :].astype(F32), axis=-1, keepdims=True) * (1.0 / D)
            mean_s[r:r + 16, :] = jnp.broadcast_to(v, (16, 128))
            return mean_s if r == order[-1] or cur["pin_stats"] else None

        def rstd(r):
            cur["tl"].hold(mean_s, lags[0])
            c = src(1)[r:r + 16, :].astype(F32) - jnp.concatenate([dyn(mean_s)[r:r + 16, :]] * ND, axis=1)
            v = jnp.sum(c * c, axis=-1, keepdims=True) * (1.0 / D)
            rstd_s[r:r + 16, :] = jnp.broadcast_to(lax.rsqrt(v + EPS), (16, 128))
            return rstd_s if r == order[-1] or cur["pin_stats"] else None

        def norm(r, ks):
            cur["tl"].hold(rstd_s, lags[1])

            def y(half, c):
                rows = slice(half * HB + r, half * HB + r + 16)
                return (src(2)[rows, _col(c)].astype(F32) - dyn(mean_s, zero)[rows, :]) * dyn(rstd_s)[rows, :]

            put_left(dst.at[_at(row0, XR, 8)], r, y, ks, n_terms)
            return dst

        return ([functools.partial(mean, r) for r in order], [functools.partial(rstd, r) for r in order],
                [functools.partial(norm, r, ks) for r in range(0, HB, 16) for ks in cur["norm"]])

    def ln1_tasks(j, times):
        sweeps = ln_tasks(lambda i: dyn(x_s, j * TB + i * zero, TB, 16), ln1_s, xn_s, j % 2 * XR, 9, cur["hold_ln1"])
        return list(zip(sweeps, times))

    def ln2_tasks(j):
        mean, rstd, norm = ln_tasks(lambda i: dyn(h_s, j * TB + i * zero, TB), ln2_s, hn_s, 0, 7, cur["hold_ln2"])
        return mean + [None] + rstd + [g for f in norm for g in (f, None)][:-1]

    def ln1_now(j):
        for r in range(0, HB, 16):
            ys = []
            for half in range(2):
                x = x_s[j * TB + half * HB + r:j * TB + half * HB + r + 16, :].astype(F32)
                c = x - jnp.sum(x, axis=-1, keepdims=True) * (1.0 / D)
                ys.append(c * lax.rsqrt(jnp.sum(c * c, axis=-1, keepdims=True) * (1.0 / D) + EPS))
            put_left(xn_s.at[pl.ds(j * XR, XR)], r, lambda half, c: ys[half][:, _col(c)], (KH, *range(KH)), 9)

    def qkv_jobs(j, i, done):
        if isinstance(j, int) and j < 2 and i == 0:
            def lhs(c, half, k, r, n):
                t = _QUADRANT[half][k // KH] * KH + k % KH if k < 2 * KH else 9 * KH + half
                return dyn(xn_s, j * XR + c * zero, XR)[_tile(t, RH, r // 2, n // 2)]
            return [job for c in range(ND) for half in range(2) for job in chain(
                ND, functools.partial(lhs, c, half), lambda k, c=c: wqkv_s[_col(k), _col(c)], lambda k: (),
                lambda: None, functools.partial(done, half, c))]
        return gemm_jobs(xn_s, j % 2 * XR, XR, i * ND, cqkv_s[i], ND, ND, done, lambda k: (("w", i),))

    def q_jobs(j):
        buf = q_s[j % 2 if isinstance(j, int) else 0]

        def done(half, c, v):
            buf[half * RH:(half + 1) * RH, _col(c)] = _pack(v * QSCALE)

        def flip(c):
            qt_s[64 * c:64 * c + 64, _at(j * TB, TB, TB)] = _u32(_bf(dyn(buf)[:, _col(c)]).T)
            return qt_s
        return qkv_jobs(j, 0, done), [functools.partial(flip, c) for c in range(ND)]

    def k_jobs(j):
        def done(half, c, v):
            k_s[_at(j * RB + half * RH + 48, RH, 8), _col(c)] = _pack(v)
        return qkv_jobs(j, 1, done)

    def v_jobs(j):
        buf = v_s[j % 2 if isinstance(j, int) else 0]
        sub = _iota((8, TB), 0)

        def done(half, c, v):
            buf[half * RH:(half + 1) * RH, _col(c)] = _pack(v)

        def flip(c):
            vp_s[64 * c:64 * c + 64, :] = _u32(_bf(dyn(buf)[:, _col(c)]).T)
            return vp_s

        def widen(c, i0):
            vt = _bf(dyn(vp_s)[64 * c + 4 * i0:64 * c + 4 * i0 + 32, :]).astype(F32)
            cols = _at(j * TB, TB, TB)
            for i in range(8):
                pair, m = divmod(16 * c + i0 + i, 5)
                t, r = vt[8 * i:8 * i + 8], 48 * pair + 8 * (m if m <= 2 else m + 1)
                if m == 2:
                    vt_s[r:r + 8, cols] = jnp.where(sub < 4, t, 1.0)
                    vt_s[r + 8:r + 16, cols] = jnp.where(sub < 4, 1.0, t)
                else:
                    vt_s[r:r + 8, cols] = t
            return vt_s

        tasks = [functools.partial(flip, c) for c in range(ND)]
        return qkv_jobs(j, 2, done), tasks + [functools.partial(widen, c, i) for c in range(ND) for i in (0, 8)]

    def skew_tasks(j):
        lane = _iota((8, 128), 1)
        cuts, lag = cur["skew_cuts"], cur["hold_skew"]

        def task(r):
            cur["tl"].hold(k_s, lag)
            src, dst = dyn(k_s, j * RB + r, 8 + 48), ks_s.at[_at(j * RB, RB, 8)]
            prev = None
            for t in range(ND):
                head = ((128 * t + lane) * 3277) >> 16
                ks = [src[16 * s:16 * s + 8, _col(t)] for s in range(4)]
                odd = (head & 1) == 1
                e = [[jnp.where(odd, ks[2 * hi + 1], ks[2 * hi]) for hi in range(2)],
                     [jnp.where(odd, ks[2 * hi], ks[2 * hi + 1]) for hi in range(2)]]
                new = [jnp.where(((head - u % 2) & 2) == 2, e[u % 2][1 - u // 2], e[u % 2][u // 2]) for u in range(4)]
                for g in range(NG):
                    t0, t1 = 80 * g // 128, (80 * g + 79) // 128
                    if t1 == t:
                        for u in range(4):
                            v = new[u] if t0 == t1 else jnp.where(lane >= 80 * g % 128, prev[u], new[u])
                            dst[r:r + 8, _col(u * NG + g)] = v
                prev = new
                if t in cuts:
                    yield ks_s

        gens = [task(r) for r in range(0, RB, 8)]
        return [functools.partial(next, gen) for gen in gens for _ in cuts]

    def wo_jobs(j):
        def done(half, c, v):
            rows = _at(j * TB + half * HB, HB, HB)
            h_s[rows, _col(c)] = x_s[rows, _col(c)].astype(F32) + v
        return gemm_jobs(o_s, 0, None, 0, co_s, ND, ND, done, lambda k: (("o", k),))

    def ffn1_jobs(buf):
        held = {}

        def done(half, c, v):
            held[half, c] = jnp.maximum(v, 0.0)
            k = c % FH
            if half == 1 and (1, k) in held and (1, FH + k) in held:
                a21, a22 = held[1, k], held[1, FH + k]
                for i, val in ((1, a21 + a22), (3, a22), (8, a21)):
                    buf[_tile(i * FH + k, RH, 0, RH)] = _pack(val)
            elif (0, k) in held and (0, FH + k) in held:
                terms = _left_terms(held[0, k], held[0, FH + k], held[1, k], held[1, FH + k])
                for i in (0, 2, 4, 5, 6, 7):
                    buf[_tile(i * FH + k, RH, 0, RH)] = _pack(terms[i])
        return gemm_jobs(hn_s, 0, None, 0, c1_s, ND, NF, done, lambda k: ("hn",), held=1)

    def ffn2_jobs(j, buf):
        def done(half, c, v):
            rows = _at(j * TB + half * HB, HB, HB)
            out_s[rows, _col(c)] = (h_s[rows, _col(c)] + v).astype(BF)
        return gemm_jobs(buf, 0, None, 0, c2_s, NF, ND, done)

    def run_round(tl, jobs):
        if len(jobs) >= 4:
            tl.round(jobs[:4], HB)
            del jobs[:4]
            return
        assert len(jobs) == 2
        n, res = HB // 2, [[], []]
        tl.round([(lambda r, m, i=i, job=job: job[0](i * n + r, m), job[1], out.append, job[3])
                  for job, out in zip(jobs, res) for i in range(2)], n)
        for job, out in zip(jobs, res):
            job[2](jnp.concatenate(out, axis=0))
        del jobs[:]

    lane32, lane16, lane8, sub8 = _iota((32, 128), 1), _iota((16, 128), 1), _iota((8, 128), 1), _iota((8, 128), 0)
    causal = _iota((32, 128), 0) <= (lane32 & 31)
    first_chunk = {1: 5, 2: 1, 3: 0}

    def scores(tl, qb, g, nk, slot):
        c_lo = first_chunk[nk]
        keys = dyn(ks_s, qb * 64 - 80 + 16 * c_lo, 16 * (9 - c_lo))

        def lhs(u, r, n):
            return keys[r // 2:(r + n) // 2, _col(u * NG + g)]

        def rhs(u):
            tiles = [jnp.zeros((8, 128), U32)] * 8
            for i in range(5):
                head = sum((16 * i + 2 * sub8 >= DH * a).astype(I32) for a in range(1, 4))
                q = qt_s[40 * g + 8 * i:40 * g + 8 * i + 8, _at(qb * 128, 128, 128)]
                tiles[(5 * g + i) % 8] = jnp.where(((head - (lane8 >> 5)) & 3) == u, q, jnp.uint32(0))
            return _bf(jnp.concatenate(tiles, axis=0))

        def done(u, s):
            ch = {c: s[32 * (c - c_lo):32 * (c - c_lo + 1)] for c in range(c_lo, 9)}
            if nk == 3:
                ch[8] = jnp.where(causal, ch[8], ch.pop(0))
            else:
                ch[8] = jnp.where(causal, ch[8], -jnp.inf)
                for c in range(c_lo, c_lo + 3):
                    ch[c] = jnp.where((lane32 >> 5) >= c_lo + 3 - c, ch[c], -jnp.inf)
            mx = None
            for c in sorted(ch):
                for r in range(0, 32, 8):
                    mx = ch[c][r:r + 8] if mx is None else jnp.maximum(mx, ch[c][r:r + 8])
                s_s[slot][32 * c - 32:32 * c, _col(u)] = ch[c]
            s_s[slot][256:264, _col(u)] = jnp.broadcast_to(jnp.max(mx, axis=0, keepdims=True), (8, 128))

        tl.round([(functools.partial(lhs, u), functools.partial(rhs, u), functools.partial(done, u), ())
                  for u in range(4)], 32 * (9 - c_lo))

    def exp_tasks(nk, slot):
        def task(u, c):
            src = dyn(s_s[slot])
            mx = jnp.concatenate([src[256:264, _col(u)]] * 4, axis=0)
            p = jnp.exp2(src[32 * c - 32:32 * c, _col(u)] - mx)
            if c == 8 and nk == 3:
                p_s[slot][0:16, _col(u)] = _pack(jnp.where(causal, 0.0, p))
                p = jnp.where(causal, p, 0.0)
            p_s[slot][16 * c:16 * c + 16, _col(u)] = _pack(p)
            return p_s[slot]
        return [functools.partial(task, u, c) for c in (8, *range(max(first_chunk[nk], 1), 8)) for u in range(4)]

    def values(tl, qb, g, nk, slot):
        tl.need({("p", slot)})

        def prob(u, c):
            if first_chunk[nk] <= c < 9:
                return dyn(p_s[slot])[16 * c:16 * c + 16, _col(u % 4)]
            return jnp.zeros((16, 128), U32)

        def shifted(a, c):
            if not first_chunk[nk] <= c < 10:
                return jnp.zeros((16, 128), U32)
            same, lower = prob(a, c), prob(a - 1, c - 1)
            return jnp.where((lane16 & 32) != 0, lower, same)

        o = [None] * 4
        for kt in range(3 - nk, 3):
            for a in range(4):
                p = [jnp.where((lane16 & 64) != 0, shifted(a - 2, c - 2), shifted(a, c))
                     for c in range(4 * kt, 4 * kt + 4)]
                v = vt_s[24 * (4 * g + a):24 * (4 * g + a + 1), _at((qb - 2 + kt) * 128, 128, 128)]
                r = _mm(v, _bf(jnp.concatenate(p, axis=0)))
                o[a] = r if o[a] is None else r + o[a]
        for a in (0, 2):
            e, f = o[a], o[a + 1]
            total = jnp.where(sub8 < 4, f[0:8], e[16:24])
            inv = pltpu.reciprocal(total, approx=True)
            inv = inv * (2.0 - total * inv)
            e, f = e * inv[4:5], f * inv[0:1]
            for i, v in enumerate([e[0:8], e[8:16], jnp.where(sub8 < 4, e[16:24], f[0:8]), f[8:16], f[16:24]]):
                t, row = divmod(80 * g + 20 * a + 8 * i, 128)
                ot_s[t][row:row + 8, _col(slot)] = v

    def o_tasks(k):
        def quad(half, l):
            return dyn(ot_s[k + l * KH])[:, _col(half)]

        def task(i):
            if k < KH:
                v, t = _left_terms(quad(0, 0), quad(0, 1), quad(1, 0), quad(1, 1))[i], i * KH + k
            else:
                v, t = quad(i, 0), 9 * KH + i
            o_s[_tile(t, RH, 0, RH)] = _u32(v.astype(BF).T)
            return o_s
        return [functools.partial(task, i) for i in range(9 if k < KH else 2)]

    def step(segments, extra=(), j=None, attn=False, prev_attn=False, first_exp=None):
        tl = cur["tl"] = _Timeline(pin, cur["chunk"], cur["turns"])
        jobs, marks, o_ready = [], [], []
        for js, *after in segments:
            jobs += js
            if after:
                marks.append((len(jobs), *after))
        total, n_steps = len(jobs), 2 * NG

        def nk(s):
            return 1 + s % 2 if isinstance(j, int) and j + s // n_steps == 0 else 3

        def live(s):
            return attn if s >= 0 else prev_attn

        span = total * HB / 4 + (sum(32 * (9 - first_chunk[nk(s)]) for s in range(n_steps)) if attn else 0)
        for tasks, (t0, t1), *key in extra:
            tl.spread(t0 * span, t1 * span, tasks, *key)
        if prev_attn:
            tl.spread(cur["o_first"], cur["o_first"] + cur["o_span"], o_tasks(KH - 1), ("o", KH - 1))
        o_free = not any(("o", 0) in job[3] for job in jobs)
        rounds = (total + 3) // 4
        cuts = _choose_cuts(jobs, n_steps, cur["even"]) if attn else [0, 4, 6, rounds] if prev_attn else [0, rounds]
        for s in range(len(cuts) - 1):
            n = cuts[s + 1] - cuts[s]
            if live(s - 1):
                t0 = tl.t + (cur["exp"][0] if s else first_exp or cur["chunk"])
                t1 = tl.t + sum(HB if len(jobs) - 4 * i >= 4 else HB // 2 for i in range(n)) + attn * cur["exp"][1]
                tl.spread(t0, max(t0, t1), exp_tasks(nk(s - 1), (s - 1) % 2), ("p", (s - 1) % 2))
            for _ in range(n):
                assert not (prev_attn and s < 2 and any(("o", 2 * KH) in job[3] for job in jobs[:4]))
                before = total - len(jobs)
                run_round(tl, jobs)
                for end, tasks, length, *key in marks:
                    if before < end <= total - len(jobs):
                        tl.spread(tl.t + cur["after"], tl.t + cur["after"] + length, tasks, *key)
                        o_free = o_free or key == ["hn"]
            if live(s - 2):
                values(tl, 2 * j + s % 2 - 2 * (s < 2), (s - 2) // 2 % NG, nk(s - 2), s % 2)
                if s == 1:
                    tl.spread(tl.t + cur["o_after"], tl.t + cur["o_after"] + 64, o_tasks(2 * KH), ("o", 2 * KH))
                o_ready += [k for k in range(KH - 1) if s - 2 == 2 * ((128 * (KH + k) + 127) // 80) + 1]
            while o_ready and o_free:
                t0 = tl.t + cur["o_after"]
                tl.spread(t0, t0 + cur["o_span"], o_tasks(o_ready.pop(0)))
            if attn:
                scores(tl, 2 * j + s % 2, s // 2, nk(s), s % 2)
        tl.run(float("inf"))

    def send(cp):
        def task():
            cp.start()
            dyn(out_s, multiple=16)[S:, _col(0)] = jnp.zeros((2 * SPARE, 128), BF)
            return out_s
        return [task], 0

    (q0, q0_flip), (q1, q1_flip), k1 = q_jobs(0), q_jobs(1), k_jobs(1)
    qkv_weights = [weight_tasks(wqkv_s, i * ND, cqkv_s[i], ND, ND) for i in range(3)]
    late_weights = (weight_tasks(wo_s, 0, co_s, ND, ND) + weight_tasks(w1_s, 0, c1_s, ND, NF)
                    + weight_tasks(w2_s, 0, c2_s, NF, ND))
    n_head, n_next = ND * 2 * head // 4 * 4, 16

    def start0(part):
        pace("start0")
        step([(q0[:n_head] if part == 0 else q0[n_head:] + q1[:n_next],)])

    def start1():
        pace("start1")
        t = cur["t"]
        step([(q1[n_next:] + k_jobs(0) + k1[:2],)],
             [(qkv_weights[1], t[0], ("w", 1)), (q0_flip, t[1]), (qkv_weights[0], t[2]), (q1_flip, t[3])])

    def start2():
        pace("start2")
        t = cur["t"]
        cut = cur["cut"]
        step([(k1[2:cut],), (*v_jobs(0), cur["v_span"]), (*v_jobs(1), cur["v_last"]), (k1[cut:],)],
             [(qkv_weights[2], t[0], ("w", 2)), *ln1_tasks(2, t[1:4]), (skew_tasks(0), t[4])])

    def proj(j):
        pace("proj")
        t = cur["t"]
        step([(*q_jobs(j), cur["q_span"]), (*v_jobs(j), cur["v_span"]), (k_jobs(j),)],
             [*ln1_tasks(j + 1, t[:3]), (skew_tasks(j - 1), t[3])])

    def attn0():
        pace("attn0")
        j, t, cut = NB - 2, cur["t"], int(len(late_weights) * cur["share"])
        step([(*q_jobs(j), cur["q_span"]), (*v_jobs(j), cur["v_span"]), (k_jobs(j),)],
             [(late_weights[:cut], t[0]), (skew_tasks(j - 1), t[1]), *ln1_tasks(j + 1, t[2:])], j=0, attn=True)

    def attn1():
        pace("attn1")
        j, t, cut = NB - 1, cur["t"], int(len(late_weights) * _PACES["attn0"]["share"])
        ready = len(late_weights) - len(weight_tasks(w2_s, 0, c2_s, NF, ND))
        mid = t[1][0] + (t[1][1] - t[1][0]) * (ready - cut) / (len(late_weights) - cut - 1)
        step([(*q_jobs(j), cur["q_span"]), (wo_jobs(0), ln2_tasks(0), cur["ln_span"], "hn"),
              (k_jobs(j), skew_tasks(j), cur["skew_span"]), (*v_jobs(j), cur["v_span"]), (ffn1_jobs(a_s[0]),)],
             [(skew_tasks(j - 1), t[0]), (late_weights[cut:ready] + [None], (t[1][0], mid), "hn"),
              (late_weights[ready:], (mid, t[1][1]))],
             j=1, attn=True, prev_attn=True, first_exp=cur["exp"][0])

    def main(j):
        pace("main")
        f2 = ffn2_jobs(j - 2, a_s[0])
        step([(f2[:cur["cut"]],), (wo_jobs(j - 1), ln2_tasks(j - 1), cur["ln_span"], "hn"),
              (f2[cur["cut"]:], [lambda: out_cp(j - 2).start()], 0), (ffn1_jobs(a_s[0]),)],
             j=j, attn=True, prev_attn=True)

    def finish():
        pace("finish")
        f2, last, (c0, c1) = ffn2_jobs(NB - 2, a_s[0]), ffn2_jobs(NB - 1, a_s[1]), cur["cut"]
        n = 7 * FH * KH
        step([(f2[:c0],), (wo_jobs(NB - 1), ln2_tasks(NB - 1), cur["ln_span"], "hn"),
              (f2[c0:c1] + ffn1_jobs(a_s[1]),), (f2[c1:], *send(out_cp(NB - 2))),
              (last[:n], *send(out_cp(NB - 1, 0, 2 * KH))), (last[n:],)], j=NB, prev_attn=True)

    def loop(lo, hi, body):
        lax.fori_loop(0, hi - lo, lambda i, carry: body(lo + zero + i), None)

    x_cp(0).wait()
    ln1_now(0)
    wk_cp.start()
    wq_head.wait()
    start0(0)
    x_cp(1).wait()
    ln1_now(1)
    wq_rest.wait()
    start0(1)
    wv_cp.start()
    x_cp(2).start()
    wk_cp.wait()
    start1()
    for i in range(3, NB):
        x_cp(i).start()
    wv_cp.wait()
    x_cp(2).wait()
    start2()
    for cp in late_cps:
        cp.start()
    for i in range(3, NB):
        x_cp(i).wait()
    loop(2, NB - 2, proj)
    for cp in late_cps:
        cp.wait()
    attn0()
    attn1()
    loop(2, NB, main)
    finish()
    out_cp(NB - 1, 2 * KH, ND).start()
    for i in range(NB - 1):
        out_cp(i).wait()
    out_cp(NB - 1, 0, 2 * KH).wait()
    out_cp(NB - 1, 2 * KH, ND).wait()


def _layer(x, wqkv, wo, w1, w2):
    (S, D), FF = x.shape, w1.shape[1]
    nd, nf = D // 128, FF // 128
    vmem = pltpu.VMEM

    def tiled(count, rows, dtype=U32, blocks=1):
        return vmem((blocks * -(-count // 4) * rows + SPARE, 512), dtype)

    def right(nk, nn):
        return tiled(7 * (nk // 2) * (nn // 2) + nk * nn - nk // 2 * 2 * (nn // 2 * 2), 64)

    left = 9 * (nd // 2) + 2
    stats = [vmem((TB + 32, 128), F32)] * 2
    hbm = pl.BlockSpec(memory_space=pl.ANY)
    return pl.pallas_call(
        _kernel,
        in_specs=[hbm] * 5,
        out_specs=hbm,
        out_shape=jax.ShapeDtypeStruct((S, D), x.dtype),
        scratch_shapes=[
            vmem((S, D), BF), vmem((D, 3 * D), BF), vmem((D, D), BF), vmem((D, FF), BF), vmem((FF, D), BF),
            [right(nd, nd)] * 3, right(nd, nd), right(nd, nf), right(nf, nd), stats, stats,
            tiled(left, RH, blocks=2), [vmem((RB, D), U32)] * 2, [vmem((RB, D), U32)] * 2,
            vmem((D // 2 + 16, TB), U32), vmem((D // 2 + SPARE, S), U32), vmem((S // 2 + 64, D), U32),
            vmem((S // 2 + SPARE, 128 * H), U32), vmem((24 * H + SPARE, S), F32),
            [vmem((264, 512), F32)] * 2, [vmem((144 + SPARE, 512), U32)] * 2, [vmem((128, TB), F32)] * nd,
            tiled(left, RH), vmem((S, D), F32), tiled(left, RH), [tiled(9 * (nf // 2), RH)] * 2,
            vmem((S + 2 * SPARE, D), BF),
            pltpu.SemaphoreType.DMA((7,)), pltpu.SemaphoreType.DMA((S // TB,)), pltpu.SemaphoreType.DMA((S // TB + 1,)),
        ],
        compiler_params=pltpu.CompilerParams(vmem_limit_bytes=100 << 20),
        name="fused_layer",
    )(x, wqkv, wo, w1, w2)


@jax.jit
def pallas_sequential_preLN__sliding_block__dense_activation_relu__prompt_kernel(
    A_x: jax.Array,
    A_wqkv: jax.Array,
    A_wo: jax.Array,
    B_x: jax.Array,
    B_w1: jax.Array,
    B_w2: jax.Array,
):
    del B_x
    return _layer(A_x.reshape(A_x.shape[-2:]), A_wqkv, A_wo, B_w1, B_w2).reshape(A_x.shape)
```

```python
import functools
import heapq

import jax
import jax.numpy as jnp
import numpy as np
from jax import lax
from jax.experimental import pallas as pl
from jax.experimental.pallas import tpu as pltpu

BF, F32, U32, I32 = jnp.bfloat16, jnp.float32, jnp.uint32, jnp.int32
H, DH = 32, 20
NG = H // 4
TB = 256
HB = TB // 2
RB, RH = TB // 2, HB // 2
SPARE = 8
EPS = 1e-5
QSCALE = float(DH ** -0.5 * np.log2(np.e))

_PACE = dict(chunk=16, turns=1, even=1.5, after=300, exp=(192, 96), o_first=288, o_after=600, o_span=1000,
             q_span=900, v_span=1000, pin_stats=True, norm=((0, 1, 2),), hold_ln1=(512, 224), hold_ln2=(512, 256),
             hold_skew=224, q_parts=True, skew_cuts=(2, 4))
_PACES = dict(
    start0=dict(),
    start1=dict(chunk=32, n_k=38, q_span=800, t=((0.1, 0.25), (0.3, 0.47), (0.55, 0.98), (0.55, 0.98))),
    start2=dict(chunk=32, cut=56, v_last=300, v_span=600, pin_stats=False, after=500, norm=((0,), (1, 2)),
                t=((0.0, 0.07), (0.08, 0.175), (0.2, 0.36), (0.4, 0.48), (0.46, 0.66), (0.72, 0.96)),
                hold_ln1=(400, 224)),
    proj=dict(after=550, q_span=200, v_span=300, pin_stats=False, hold_ln1=(600, 224), norm=((0,), (1,), (2,)),
              skew_cuts=(1, 2, 3, 4), t=((0.05, 0.12), (0.13, 0.27), (0.425, 0.8), (0.2, 0.75)), hold_skew=256),
    attn0=dict(turns=2, even=5, after=500, o_span=2000, pin_stats=False, v_span=800, norm=((0,), (1,), (2,)),
               share=0.33, t=((0.02, 0.99), (0.03, 0.08), (0.12, 0.28), (0.25, 0.6)), o_after=800, hold_ln1=(600, 224)),
    attn1=dict(turns=2, even=3, after=400, q_span=1000, v_span=600, skew_cuts=(0, 1, 2, 3, 4), ln_span=3200,
               skew_span=3500, t=((0.01, 0.33), (0.02, 0.97)), q_parts=False, norm=((0,), (1, 2)), pin_stats=False),
    main=dict(cut=44, ln_span=2200),
    finish=dict(cut=(40, 100), ln_span=1500),
)


def _mm(a, b):
    return lax.dot_general(a, b, (((1,), (0,)), ((), ())), preferred_element_type=F32)


def _iota(shape, d):
    return lax.broadcasted_iota(I32, shape, d)


def _at(start, n, multiple):
    return pl.ds(start if isinstance(start, int) else pl.multiple_of(start, multiple), n)


def _u32(x):
    return pltpu.bitcast(x, U32)


def _bf(x):
    return pltpu.bitcast(x, BF)


def _pack(x):
    return _u32(x.astype(BF))


def _col(c, n=1):
    return slice(128 * c, 128 * (c + n))


def _tile(i, rows, r, n):
    return slice(i // 4 * rows + r, i // 4 * rows + r + n), _col(i % 4)


def _left_terms(a11, a12, a21, a22):
    return [a11 + a22, a21 + a22, a11, a22, a11 + a12, a21 - a11, a12 - a22, a12, a21]


def _right_terms(b11, b12, b21, b22):
    return [b11 + b22, b11, b12 - b22, b21 - b11, b22, b11 + b12, b21 + b22]


_QUADRANT = ((2, 7), (8, 3))


def _choose_cuts(jobs, n, even):
    rounds = (len(jobs) + 3) // 4
    open_at = [0] + [jobs[min(4 * r, len(jobs)) - 1][4] for r in range(1, rounds + 1)]
    best = {0: (0.0, [0])}
    for _ in range(n):
        best = {r: min((cost + open_at[r] + even * (r - p - rounds / n) ** 2, path + [r])
                       for p, (cost, path) in best.items() if p < r)
                for r in range(min(best) + 1, rounds + 1)}
    return best[rounds][1]


class _Timeline:
    def __init__(self, pin, chunk, turns):
        self.pin, self.chunk, self.turns = pin, chunk, turns
        self.t = self.now = self.count = self.turn = 0
        self.queue, self.stored, self.results = [], {}, []

    def spread(self, t0, t1, tasks, key=None):
        for i, task in enumerate(tasks):
            if task is not None:
                heapq.heappush(self.queue, (t0 + (t1 - t0) * i / max(len(tasks) - 1, 1), self.count, task, key))
                self.count += 1

    def run(self, t):
        self.now = t
        while self.queue and self.queue[0][0] <= t:
            ref = heapq.heappop(self.queue)[2]()
            if ref is not None:
                self.stored[id(ref)] = ref

    def need(self, keys):
        due = sorted(e for e in self.queue if e[3] in keys)
        self.queue = [e for e in self.queue if e[3] not in keys]
        heapq.heapify(self.queue)
        for e in due:
            e[2]()

    def hold(self, ref, lag):
        old = [v for t, v in self.results if t <= self.now - lag]
        if old:
            ref[ref.shape[0] - SPARE:, _col(0)] = old[-1] if ref.dtype == F32 else _u32(old[-1])

    def round(self, jobs, rows):
        parts = [[] for _ in jobs]
        self.need({k for job in jobs for k in job[3]})
        for r in range(0, rows, self.chunk):
            self.run(self.t + r)
            for p, job in zip(parts, jobs):
                p.append(job[0](r, self.chunk))
            for ref in self.stored.values():
                self.turn = (self.turn + 1) % self.turns
                parts[self.turn][-1] = self.pin(parts[self.turn][-1], ref)
            self.stored = {}
        for p, job in zip(parts, jobs):
            res = _mm(_bf(jnp.concatenate(p, axis=0)), job[1]())
            out = job[2](res)
        out = res if out is None else out
        self.results += [(self.t + r, out[r:r + SPARE]) for r in range(0, rows, self.chunk)]
        self.t += rows


def _kernel(x_hbm, wqkv_hbm, wo_hbm, w1_hbm, w2_hbm, out_hbm,
            x_s, wqkv_s, wo_s, w1_s, w2_s, cqkv_s, co_s, c1_s, c2_s, ln1_s, ln2_s, xn_s, qh_s, q_s, v_s, vp_s,
            qt_s, k_s, ks_s, vt_s, s_s, p_s, ot_s, o_s, h_s, hn_s, a_s, out_s, sem_w, sem_x, sem_out):
    (S, D), FF = x_hbm.shape, w1_hbm.shape[1]
    NB, ND, NF = S // TB, D // 128, FF // 128
    KH, FH = ND // 2, NF // 2
    PAIR = 7 * KH + 4
    XR = o_s.shape[0] - SPARE
    cur = {}

    def pace(name):
        cur.update(_PACE, **_PACES[name])

    def x_cp(i, n=1):
        at = _at(i * TB, n * TB, TB)
        return pltpu.make_async_copy(x_hbm.at[at], x_s.at[at], sem_x.at[i])

    out_parts = ((slice(0, S - 2 * TB), _col(0, ND)), (slice(S - 2 * TB, S - TB), _col(0, ND)),
                 (slice(S - TB, S), _col(0, 2 * KH)), (slice(S - TB, S), _col(2 * KH)))
    out_cps = [pltpu.make_async_copy(out_s.at[at], out_hbm.at[at], sem_out.at[i]) for i, at in enumerate(out_parts)]

    head = qh_s.shape[1] // 128
    qkv_cols = (0, ND, 2 * ND - 1, 3 * ND)
    wq_head, wq_rest, wk_cp, wv_cp = [
        pltpu.make_async_copy(wqkv_hbm.at[:, _col(c0, c1 - c0)], wqkv_s.at[:, _col(c0, c1 - c0)], sem_w.at[i])
        for i, (c0, c1) in enumerate(((0, head), (head, ND), qkv_cols[1:3], qkv_cols[2:]))]
    late_cps = [pltpu.make_async_copy(src, dst, sem_w.at[4 + i])
                for i, (src, dst) in enumerate(((wo_hbm, wo_s), (w1_hbm, w1_s), (w2_hbm, w2_s)))]
    for cp in (x_cp(0), wq_head, x_cp(1), wq_rest):
        cp.start()

    k_s[0:48, :] = jnp.zeros((48, D), U32)
    for ref in (*cqkv_s, co_s, c1_s, c2_s, *ln1_s, *ln2_s, xn_s, vp_s, qt_s, ks_s, vt_s, *p_s, o_s, hn_s):
        ref[ref.shape[0] - SPARE:, _col(0)] = jnp.zeros((SPARE, 128), ref.dtype)

    zero = lax.fori_loop(0, 2, lambda i, c: i * (i - 1) * (2 * i - 1) * 128, jnp.int32(0))
    keep = _iota((8, 128), 0) >= zero

    def dyn(ref, row=0, n=None, multiple=8):
        return ref.at[_at(zero + row, n or ref.shape[0], multiple)]

    def pin(v, ref):
        n = 2 * SPARE if ref.dtype == BF else SPARE
        w = dyn(ref, multiple=n)[ref.shape[0] - n:, _col(0)]
        first = jnp.where(keep, v[0:8], w if w.dtype == U32 else _u32(w))
        return jnp.concatenate([first, v[8:]], axis=0) if v.shape[0] > 8 else first

    def chain(n, lhs, rhs, key, start, finish, live=(1, 0)):
        acc = []

        def done(r):
            prev = acc[-1] if acc else start()
            acc.append(r if prev is None else r + prev)
            if len(acc) == n:
                finish(acc[-1])
            return acc[-1]
        return [(functools.partial(lhs, k), functools.partial(rhs, k), done, key(k), live[k == n - 1])
                for k in range(n)]

    def gemm_jobs(a_ref, row0, rows, tag, c_ref, nk, nn, done, key=lambda k, c: (), held=0):
        kh, nh, odd = nk // 2, nn // 2, nk % 2
        none = lambda: None

        def left(c, term, k, r, n):
            return dyn(a_ref, row0 + (tag + c) * zero, rows)[_tile(term * kh + k, RH, r // 2, n // 2)]

        def plain_left(c, half, k, r, n):
            if k < 2 * kh:
                return left(c, _QUADRANT[half][k // kh], k % kh, r, n)
            return left(c, 9, half, r, n)

        def right(i):
            return _bf(dyn(c_ref)[_tile(i, 64, 0, 64)])

        jobs = []
        for c in range(nh):
            v = {}

            def prod(term, start, finish, live, c=c):
                return chain(kh, functools.partial(left, c, term), lambda k: right((term * kh + k) * nh + c),
                             lambda k: key(k, c) + key(kh + k, c), start, finish, live)

            def rest(half, cc, start, finish, live):
                return chain(odd, lambda k, r, n: plain_left(cc, half, 2 * kh, r, n),
                             lambda k: right(7 * kh * nh + cc), lambda k: key(2 * kh, cc % nh), start, finish,
                             (live, live))

            def m2(m, v=v):
                v["c21"] = v["m2"] = m

            def m4(m, v=v, c=c):
                done(1, c, m + v["c21"])
                v["m4"] = m

            def m1(m, v=v):
                v["c11"], v["c22"] = m + v["m4"], m + v["c22"] if odd else m - v["m2"]

            def m3(m, v=v, c=c):
                done(1, nh + c, m + v["c22"])
                v["c12"] = m

            def m5(m, v=v, c=c):
                v["c11"], v["c12"] = v["c11"] - m, v["c12"] + m
                if not odd:
                    done(0, nh + c, v["c12"])

            def m7(m, v=v, c=c):
                v["c11"] = m
                if not odd:
                    done(0, c, m)

            get = lambda name, v=v: (lambda: v[name])
            put = lambda name, v=v: (lambda m: v.update({name: m}))
            e = held
            jobs += prod(1, none, m2, (1, 1))
            jobs += rest(1, c, get("c21"), put("c21"), 2)
            jobs += rest(1, nh + c, none, lambda m, v=v: v.update(c22=m - v["m2"]), 2)
            jobs += prod(3, none, m4, (2 + odd, 2 + e)) + prod(0, none, m1, (3 + e, 2 + e))
            jobs += prod(5, get("c22"), put("c22"), (2 + e, 2 + e)) + prod(2, none, m3, (3 + e, 2 + 2 * e))
            jobs += prod(4, none, m5, (3 + 2 * e, 2 + 2 * e)) + prod(6, get("c11"), m7, (2 + 2 * e, 2 * odd + 2 * e))
            jobs += rest(0, c, get("c11"), functools.partial(done, 0, c), 2 + 2 * e)
            jobs += rest(0, nh + c, get("c12"), functools.partial(done, 0, nh + c), 0)
        for c in range(2 * nh, nn):
            for half in range(2):
                jobs += chain(nk, functools.partial(plain_left, c, half),
                              lambda k: right(7 * kh * nh + odd * 2 * nh + k), lambda k: key(k, nh), none,
                              functools.partial(done, half, c))
        return jobs

    def weight_tasks(w_ref, col0, c_ref, nk, nn, pair=None):
        kh, nh = nk // 2, nn // 2

        def combine(k, r, c):
            b = [w_ref[128 * (i * kh + k) + r:128 * (i * kh + k) + r + 16, _col(col0 + l * nh + c)]
                 for i in range(2) for l in range(2)]
            for term, val in enumerate(_right_terms(*[t.astype(F32) for t in b])):
                val = _u32(b[0]) if term == 1 else _u32(b[3]) if term == 4 else _pack(val)
                c_ref[_tile((term * kh + k) * nh + c, 64, r // 2, 8)] = val
            return c_ref

        def copy(i, k, c):
            c_ref[_tile(7 * kh * nh + i, 64, 0, 64)] = _u32(w_ref[_col(k), _col(col0 + c)])
            return c_ref

        rest = [(k, c) for k in range(2 * kh, nk) for c in range(2 * nh)]
        rest += [(k, c) for c in range(2 * nh, nn) for k in range(nk)]
        return ([functools.partial(combine, k, r, c) for c in range(nh) for k in range(kh) for r in range(0, 128, 16)
                 if pair in (None, c)]
                + [functools.partial(copy, i, k, c) for i, (k, c) in enumerate(rest) if pair in (None, c % nh)])

    def put_left(out, r, y, ks, n_terms):
        for k in ks:
            if k < KH:
                terms = _left_terms(y(0, k), y(0, KH + k), y(1, k), y(1, KH + k))
                for i in range(n_terms):
                    out[_tile(i * KH + k, RH, r // 2, 8)] = _pack(terms[i])
            else:
                for half in range(2):
                    out[_tile(9 * KH + half, RH, r // 2, 8)] = _pack(y(half, 2 * KH))

    def ln_tasks(src, stats, dst, row0, n_terms, lags):
        mean_s, rstd_s = stats
        order = [half * HB + r for r in range(0, HB, 16) for half in range(2)]

        def mean(r):
            v = jnp.sum(src(0)[r:r + 16, :].astype(F32), axis=-1, keepdims=True) * (1.0 / D)
            mean_s[r:r + 16, :] = jnp.broadcast_to(v, (16, 128))
            return mean_s if r == order[-1] or cur["pin_stats"] else None

        def rstd(r):
            cur["tl"].hold(mean_s, lags[0])
            c = src(1)[r:r + 16, :].astype(F32) - jnp.concatenate([dyn(mean_s)[r:r + 16, :]] * ND, axis=1)
            v = jnp.sum(c * c, axis=-1, keepdims=True) * (1.0 / D)
            rstd_s[r:r + 16, :] = jnp.broadcast_to(lax.rsqrt(v + EPS), (16, 128))
            return rstd_s if r == order[-1] or cur["pin_stats"] else None

        def norm(r, ks):
            cur["tl"].hold(rstd_s, lags[1])

            def y(half, c):
                rows = slice(half * HB + r, half * HB + r + 16)
                return (src(2)[rows, _col(c)].astype(F32) - dyn(mean_s, zero)[rows, :]) * dyn(rstd_s)[rows, :]

            put_left(dst.at[_at(row0, XR, 8)], r, y, ks, n_terms)
            return dst

        return ([functools.partial(mean, r) for r in order], [functools.partial(rstd, r) for r in order],
                [functools.partial(norm, r, ks) for r in range(0, HB, 16) for ks in cur["norm"]])

    def ln1_tasks(j, times):
        sweeps = ln_tasks(lambda i: dyn(x_s, j * TB + i * zero, TB, 16), ln1_s, xn_s, j % 2 * XR, 9, cur["hold_ln1"])
        return list(zip(sweeps, times))

    def ln2_tasks(j):
        mean, rstd, norm = ln_tasks(lambda i: dyn(h_s, j * TB + i * zero, TB), ln2_s, hn_s, 0, 7, cur["hold_ln2"])
        return mean + [None] + rstd + [g for f in norm for g in (f, None)][:-1]

    def ln1_now(j):
        src, dst = x_s.at[_at(j * TB, TB, TB)], xn_s.at[_at(j * XR, XR, 8)]
        for r in range(0, HB, 16):
            ys = []
            for half in range(2):
                x = src[half * HB + r:half * HB + r + 16, :].astype(F32)
                c = x - jnp.sum(x, axis=-1, keepdims=True) * (1.0 / D)
                ys.append(c * lax.rsqrt(jnp.sum(c * c, axis=-1, keepdims=True) * (1.0 / D) + EPS))
            put_left(dst, r, lambda half, c: ys[half][:, _col(c)], (KH, *range(KH)), 9)

    def qkv_jobs(j, i, done):
        return gemm_jobs(xn_s, j % 2 * XR, XR, i * ND, cqkv_s[i], ND, qkv_cols[i + 1] - qkv_cols[i], done,
                         lambda k, c: (("w", i, c),))

    def q_io(j, place):
        def done(half, c, v):
            buf, row, cols = place(c)
            buf[_at(row + half * RH, RH, RH), cols] = _pack(v * QSCALE)

        def flip(c):
            buf, row, cols = place(c)
            qt_s[_at(j * (D // 2) + 64 * c, 64, 64), :] = _u32(_bf(dyn(buf, row, RB)[:, cols]).T)
            return qt_s
        return done, [functools.partial(flip, c) for c in range(ND)]

    def early_q(j, cols):
        done, flips = q_io(j, lambda c: (qh_s, j * RB, _col(c)) if c < head else (q_s[j], 0, _col(c - head)))

        def lhs(c, half, k, r, n):
            t = _QUADRANT[half][k // KH] * KH + k % KH if k < 2 * KH else 9 * KH + half
            return dyn(xn_s, j * XR + c * zero, XR)[_tile(t, RH, r // 2, n // 2)]
        return [job for c in cols for half in range(2) for job in chain(
            ND, functools.partial(lhs, c, half), lambda k, c=c: wqkv_s[_col(k), _col(c)], lambda k: (),
            lambda: None, functools.partial(done, half, c))], flips

    def q_jobs(j):
        done, flips = q_io(j, lambda c: (q_s[c % KH], 0, _col(c // KH)) if c < 2 * KH else (q_s[KH], 0, _col(0)))
        jobs = qkv_jobs(j, 0, done)
        if not cur["q_parts"]:
            return [(jobs, flips, cur["q_span"])]
        return [(jobs[PAIR * i:PAIR * (i + 1)], flips[i:2 * KH:KH] if i < KH else flips[i + KH:], cur["q_span"])
                for i in range(KH + 1)]

    def put_k(j, half, c, v):
        k_s.at[_at(j * RB + half * RH, 48 + RH, RH)][48:, _col(c)] = _pack(v)

    def k_jobs(j):
        return qkv_jobs(j, 1, functools.partial(put_k, j))

    def v_jobs(j, span):
        buf = v_s[j % 2 if isinstance(j, int) else 0]
        sub = _iota((8, TB), 0)

        def done(half, c, v):
            if c == 0:
                put_k(j, half, ND - 1, v)
            else:
                buf[c % (KH + 1)][half * RH:(half + 1) * RH, _col(c // (KH + 1))] = _pack(v)

        def flip(c):
            side, pair = divmod(c + 1, KH + 1)
            vp_s[64 * c:64 * c + 64, :] = _u32(_bf(dyn(buf[pair])[:, _col(side)]).T)
            return vp_s

        def widen(c, i0):
            vt = _bf(dyn(vp_s)[64 * c + 4 * i0:64 * c + 4 * i0 + 32, :]).astype(F32)
            dst = vt_s.at[_at(j * 24 * H, 24 * H, 64)]
            for i in range(8):
                pair, m = divmod(16 * c + i0 + i, 5)
                t, r = vt[8 * i:8 * i + 8], 48 * pair + 8 * (m if m <= 2 else m + 1)
                if m == 2:
                    dst[r:r + 8, :] = jnp.where(sub < 4, t, 1.0)
                    dst[r + 8:r + 16, :] = jnp.where(sub < 4, 1.0, t)
                else:
                    dst[r:r + 8, :] = t
            return vt_s

        def tasks(cs):
            return ([functools.partial(flip, c) for c in cs]
                    + [functools.partial(widen, c, i) for c in cs for i in (0, 8)])

        jobs = qkv_jobs(j, 2, done)
        return [(jobs[PAIR * i:PAIR * (i + 1)], tasks([c for c in (i - 1, i + KH) if c >= 0]), span)
                for i in range(KH + 1)]

    def skew_tasks(j):
        lane = _iota((8, 128), 1)
        cuts, lag = cur["skew_cuts"], cur["hold_skew"]

        def task(r):
            cur["tl"].hold(k_s, lag)
            src, dst = dyn(k_s, j * RB, RB + 48), ks_s.at[_at(j * RB, RB, 8)]
            prev = None
            for t in range(ND):
                head = ((128 * t + lane) * 3277) >> 16
                ks = [src[r + 16 * s:r + 16 * s + 8, _col(t)] for s in range(4)]
                odd = (head & 1) == 1
                e = [[jnp.where(odd, ks[2 * hi + 1], ks[2 * hi]) for hi in range(2)],
                     [jnp.where(odd, ks[2 * hi], ks[2 * hi + 1]) for hi in range(2)]]
                new = [jnp.where(((head - u % 2) & 2) == 2, e[u % 2][1 - u // 2], e[u % 2][u // 2]) for u in range(4)]
                for g in range(NG):
                    t0, t1 = 80 * g // 128, (80 * g + 79) // 128
                    if t1 == t:
                        for u in range(4):
                            v = new[u] if t0 == t1 else jnp.where(lane >= 80 * g % 128, prev[u], new[u])
                            dst[r:r + 8, _col(4 * g + u)] = v
                prev = new
                if t in cuts:
                    yield ks_s

        gens = [task(r) for r in range(0, RB, 8)]
        return [functools.partial(next, gen) for gen in gens for _ in cuts]

    def wo_jobs(j):
        def done(half, c, v):
            rows = _at(j * TB + half * HB, HB, HB)
            h_s[rows, _col(c)] = x_s[rows, _col(c)].astype(F32) + v
        return gemm_jobs(o_s, 0, None, 0, co_s, ND, ND, done, lambda k, c: (("o", k),))

    def ffn1_jobs(buf):
        held = {}

        def done(half, c, v):
            held[half, c] = jnp.maximum(v, 0.0)
            k = c % FH
            if half == 1 and (1, k) in held and (1, FH + k) in held:
                a21, a22 = held[1, k], held[1, FH + k]
                for i, val in ((1, a21 + a22), (3, a22), (8, a21)):
                    buf[_tile(i * FH + k, RH, 0, RH)] = _pack(val)
            elif (0, k) in held and (0, FH + k) in held:
                terms = _left_terms(held[0, k], held[0, FH + k], held[1, k], held[1, FH + k])
                for i in (0, 2, 4, 5, 6, 7):
                    buf[_tile(i * FH + k, RH, 0, RH)] = _pack(terms[i])
        return gemm_jobs(hn_s, 0, None, 0, c1_s, ND, NF, done, lambda k, c: ("hn",), held=1)

    def ffn2_jobs(j, buf):
        def done(half, c, v):
            rows = _at(j * TB + half * HB, HB, HB)
            out_s[rows, _col(c)] = (h_s[rows, _col(c)] + v).astype(BF)
        return gemm_jobs(buf, 0, None, 0, c2_s, NF, ND, done)

    def run_round(tl, jobs):
        if len(jobs) >= 4:
            tl.round(jobs[:4], HB)
            del jobs[:4]
            return
        assert len(jobs) == 2
        n, res = HB // 2, [[], []]
        tl.round([(lambda r, m, i=i, job=job: job[0](i * n + r, m), job[1], out.append, job[3])
                  for job, out in zip(jobs, res) for i in range(2)], n)
        for job, out in zip(jobs, res):
            job[2](jnp.concatenate(out, axis=0))
        del jobs[:]

    lane32, lane16, lane8, sub8 = _iota((32, 128), 1), _iota((16, 128), 1), _iota((8, 128), 1), _iota((8, 128), 0)
    causal = _iota((32, 128), 0) <= (lane32 & 31)
    first_chunk = {1: 5, 2: 1, 3: 0}

    def scores(tl, j, g, nk, slot):
        c_lo = first_chunk[nk]
        keys = dyn(ks_s, (2 * j + slot) * 64 - 80 + 16 * c_lo, 16 * (9 - c_lo))

        def lhs(u, r, n):
            return keys[r // 2:(r + n) // 2, _col(4 * g + u)]

        def rhs(u):
            tiles = [jnp.zeros((8, 128), U32)] * 8
            for i in range(5):
                head = sum((16 * i + 2 * sub8 >= DH * a).astype(I32) for a in range(1, 4))
                q = qt_s.at[_at(j * (D // 2), D // 2, 64)][40 * g + 8 * i:40 * g + 8 * i + 8, _col(slot)]
                tiles[(5 * g + i) % 8] = jnp.where(((head - (lane8 >> 5)) & 3) == u, q, jnp.uint32(0))
            return _bf(jnp.concatenate(tiles, axis=0))

        def done(u, s):
            ch = {c: s[32 * (c - c_lo):32 * (c - c_lo + 1)] for c in range(c_lo, 9)}
            if nk == 3:
                ch[8] = jnp.where(causal, ch[8], ch.pop(0))
            else:
                ch[8] = jnp.where(causal, ch[8], -jnp.inf)
                for c in range(c_lo, c_lo + 3):
                    ch[c] = jnp.where((lane32 >> 5) >= c_lo + 3 - c, ch[c], -jnp.inf)
            mx = None
            for c in sorted(ch):
                for r in range(0, 32, 8):
                    mx = ch[c][r:r + 8] if mx is None else jnp.maximum(mx, ch[c][r:r + 8])
                s_s[slot][32 * c - 32:32 * c, _col(u)] = ch[c]
            s_s[slot][256:264, _col(u)] = jnp.broadcast_to(jnp.max(mx, axis=0, keepdims=True), (8, 128))

        tl.round([(functools.partial(lhs, u), functools.partial(rhs, u), functools.partial(done, u), ())
                  for u in range(4)], 32 * (9 - c_lo))

    def exp_tasks(nk, slot):
        def task(u, c):
            src = dyn(s_s[slot])
            mx = jnp.concatenate([src[256:264, _col(u)]] * 4, axis=0)
            p = jnp.exp2(src[32 * c - 32:32 * c, _col(u)] - mx)
            if c == 8 and nk == 3:
                p_s[slot][0:16, _col(u)] = _pack(jnp.where(causal, 0.0, p))
                p = jnp.where(causal, p, 0.0)
            p_s[slot][16 * c:16 * c + 16, _col(u)] = _pack(p)
            return p_s[slot]
        return [functools.partial(task, u, c) for c in (8, *range(max(first_chunk[nk], 1), 8)) for u in range(4)]

    def values(tl, j, g, nk, slot):
        tl.need({("p", slot)})

        def prob(u, c):
            if first_chunk[nk] <= c < 9:
                return dyn(p_s[slot])[16 * c:16 * c + 16, _col(u % 4)]
            return jnp.zeros((16, 128), U32)

        def shifted(a, c):
            if not first_chunk[nk] <= c < 10:
                return jnp.zeros((16, 128), U32)
            same, lower = prob(a, c), prob(a - 1, c - 1)
            return jnp.where((lane16 & 32) != 0, lower, same)

        o = [None] * 4
        for kt in range(3 - nk, 3):
            for a in range(4):
                p = [jnp.where((lane16 & 64) != 0, shifted(a - 2, c - 2), shifted(a, c))
                     for c in range(4 * kt, 4 * kt + 4)]
                dj, half = divmod(slot - 2 + kt, 2)
                v = vt_s.at[_at((j + dj) * 24 * H, 24 * H, 64)][24 * (4 * g + a):24 * (4 * g + a + 1), _col(half)]
                r = _mm(v, _bf(jnp.concatenate(p, axis=0)))
                o[a] = r if o[a] is None else r + o[a]
        for a in (0, 2):
            e, f = o[a], o[a + 1]
            total = jnp.where(sub8 < 4, f[0:8], e[16:24])
            inv = pltpu.reciprocal(total, approx=True)
            inv = inv * (2.0 - total * inv)
            e, f = e * inv[4:5], f * inv[0:1]
            for i, v in enumerate([e[0:8], e[8:16], jnp.where(sub8 < 4, e[16:24], f[0:8]), f[8:16], f[16:24]]):
                t, row = divmod(80 * g + 20 * a + 8 * i, 128)
                ot_s[t][row:row + 8, _col(slot)] = v

    def o_tasks(k):
        def quad(half, l):
            return dyn(ot_s[k + l * KH])[:, _col(half)]

        def task(i):
            if k < KH:
                v, t = _left_terms(quad(0, 0), quad(0, 1), quad(1, 0), quad(1, 1))[i], i * KH + k
            else:
                v, t = quad(i, 0), 9 * KH + i
            o_s[_tile(t, RH, 0, RH)] = _u32(v.astype(BF).T)
            return o_s
        return [functools.partial(task, i) for i in range(9 if k < KH else 2)]

    def step(segments, extra=(), j=None, attn=False, prev_attn=False, first_exp=None):
        tl = cur["tl"] = _Timeline(pin, cur["chunk"], cur["turns"])
        jobs, marks, o_ready = [], [], []
        for js, *after in segments:
            jobs += js
            if after:
                marks.append((len(jobs), *after))
        total, n_steps = len(jobs), 2 * NG

        def nk(s):
            return 1 + s % 2 if isinstance(j, int) and j + s // n_steps == 0 else 3

        def live(s):
            return attn if s >= 0 else prev_attn

        span = total * HB / 4 + (sum(32 * (9 - first_chunk[nk(s)]) for s in range(n_steps)) if attn else 0)
        for tasks, (t0, t1), *key in extra:
            tl.spread(t0 * span, t1 * span, tasks, *key)
        if prev_attn:
            tl.spread(cur["o_first"], cur["o_first"] + cur["o_span"], o_tasks(KH - 1), ("o", KH - 1))
        o_free = not any(("o", 0) in job[3] for job in jobs)
        rounds = (total + 3) // 4
        cuts = _choose_cuts(jobs, n_steps, cur["even"]) if attn else [0, 4, 6, rounds] if prev_attn else [0, rounds]
        for s in range(len(cuts) - 1):
            n = cuts[s + 1] - cuts[s]
            if live(s - 1):
                t0 = tl.t + (cur["exp"][0] if s else first_exp or cur["chunk"])
                t1 = tl.t + sum(HB if len(jobs) - 4 * i >= 4 else HB // 2 for i in range(n)) + attn * cur["exp"][1]
                tl.spread(t0, max(t0, t1), exp_tasks(nk(s - 1), (s - 1) % 2), ("p", (s - 1) % 2))
            for _ in range(n):
                assert not (prev_attn and s < 2 and any(("o", 2 * KH) in job[3] for job in jobs[:4]))
                before = total - len(jobs)
                run_round(tl, jobs)
                for end, tasks, length, *key in marks:
                    if before < end <= total - len(jobs):
                        tl.spread(tl.t + cur["after"], tl.t + cur["after"] + length, tasks, *key)
                        o_free = o_free or key == ["hn"]
            if live(s - 2):
                values(tl, j - (s < 2), (s - 2) // 2 % NG, nk(s - 2), s % 2)
                if s == 1:
                    tl.spread(tl.t + cur["o_after"], tl.t + cur["o_after"] + 64, o_tasks(2 * KH), ("o", 2 * KH))
                o_ready += [k for k in range(KH - 1) if s - 2 == 2 * ((128 * (KH + k) + 127) // 80) + 1]
            while o_ready and o_free:
                t0 = tl.t + cur["o_after"]
                tl.spread(t0, t0 + cur["o_span"], o_tasks(o_ready.pop(0)))
            if attn:
                scores(tl, j, s // 2, nk(s), s % 2)
        tl.run(float("inf"))

    def send(cp):
        def task():
            cp.start()
            dyn(out_s, multiple=16)[S:, _col(0)] = jnp.zeros((2 * SPARE, 128), BF)
            return out_s
        return [task], 0

    k01, n_k = k_jobs(0) + k_jobs(1), _PACES["start1"]["n_k"]

    def qkv_weights(i, times):
        c0, c1 = qkv_cols[i:i + 2]
        return [(weight_tasks(wqkv_s, c0, cqkv_s[i], ND, c1 - c0, c if i else None), t, ("w", i, c))
                for c, t in enumerate(times)]

    late_weights = (weight_tasks(wo_s, 0, co_s, ND, ND) + weight_tasks(w1_s, 0, c1_s, ND, NF)
                    + weight_tasks(w2_s, 0, c2_s, NF, ND))

    def start0(j):
        x_cp(j).wait()
        ln1_now(j)
        for i, (ahead, needed) in enumerate(((wk_cp, wq_head), (wv_cp, wq_rest))):
            @pl.when(j == i)
            def _():
                ahead.start()
                needed.wait()
        pace("start0")
        step([(early_q(j, range(head))[0],)])

    def start1():
        pace("start1")
        t, ((q0, q0_flip), (q1, q1_flip)) = cur["t"], (early_q(j, range(head, ND)) for j in range(2))
        step([(q0, q0_flip[head:], cur["q_span"]), (q1, q1_flip[head:], cur["q_span"]), (k01[:n_k],)],
             [*qkv_weights(1, t[:2]), (q0_flip[:head] + q1_flip[:head], t[2]), *qkv_weights(0, t[3:])])

    def start2():
        pace("start2")
        t = cur["t"]
        cut = cur["cut"]
        step([(k01[n_k:cut],), *v_jobs(0, cur["v_span"]), *v_jobs(1, cur["v_last"]), (k01[cut:],)],
             [*qkv_weights(2, t[:3]), *ln1_tasks(2, t[3:])])

    def proj(j):
        pace("proj")
        t = cur["t"]
        step([*v_jobs(j, cur["v_span"]), *q_jobs(j), (k_jobs(j),)],
             [*ln1_tasks(j + 1, t[:3]), (skew_tasks(j - 2), t[3])])

    def attn0():
        pace("attn0")
        j, t, cut = NB - 2, cur["t"], int(len(late_weights) * cur["share"])
        step([*q_jobs(j), *v_jobs(j, cur["v_span"]), (k_jobs(j),)],
             [(late_weights[:cut], t[0]), *ln1_tasks(j + 1, t[1:])], j=0, attn=True)

    def attn1():
        pace("attn1")
        j, t, cut = NB - 1, cur["t"], int(len(late_weights) * _PACES["attn0"]["share"])
        ready = len(late_weights) - len(weight_tasks(w2_s, 0, c2_s, NF, ND))
        mid = t[1][0] + (t[1][1] - t[1][0]) * (ready - cut) / (len(late_weights) - cut - 1)
        v = v_jobs(j, cur["v_span"])
        step([*q_jobs(j), (wo_jobs(0), ln2_tasks(0), cur["ln_span"], "hn"), (k_jobs(j),), v[0],
              ([], skew_tasks(j), cur["skew_span"]), *v[1:], (ffn1_jobs(a_s[0]),)],
             [([f for i in range(j - 3, j) for f in skew_tasks(i)], t[0]),
              (late_weights[cut:ready] + [None], (t[1][0], mid), "hn"), (late_weights[ready:], (mid, t[1][1]))],
             j=1, attn=True, prev_attn=True, first_exp=cur["exp"][0])

    def main(j):
        pace("main")
        f2 = ffn2_jobs(j - 2, a_s[0])
        step([(f2[:cur["cut"]],), (wo_jobs(j - 1), ln2_tasks(j - 1), cur["ln_span"], "hn"),
              (f2[cur["cut"]:] + ffn1_jobs(a_s[0]),)], j=j, attn=True, prev_attn=True)

    def finish():
        pace("finish")
        f2, last, (c0, c1) = ffn2_jobs(NB - 2, a_s[0]), ffn2_jobs(NB - 1, a_s[1]), cur["cut"]
        n = 7 * FH * KH
        step([(f2[:c0], *send(out_cps[0])), (wo_jobs(NB - 1), ln2_tasks(NB - 1), cur["ln_span"], "hn"),
              (f2[c0:c1] + ffn1_jobs(a_s[1]),), (f2[c1:], *send(out_cps[1])),
              (last[:n], *send(out_cps[2])), (last[n:],)], j=NB, prev_attn=True)

    def loop(lo, hi, body):
        lax.fori_loop(0, hi - lo, lambda i, carry: body(lo + zero + i), None)

    loop(0, 2, start0)
    x_cp(2).start()
    wk_cp.wait()
    start1()
    x_cp(3, NB - 3).start()
    wv_cp.wait()
    x_cp(2).wait()
    start2()
    for cp in late_cps:
        cp.start()
    x_cp(3, NB - 3).wait()
    loop(0, NB // 2 - 2, lambda i: proj(2 * i + 2) or proj(2 * i + 3))
    for cp in late_cps:
        cp.wait()
    attn0()
    attn1()
    loop(2, NB, main)
    finish()
    out_cps[3].start()
    for cp in out_cps:
        cp.wait()


def _layer(x, wqkv, wo, w1, w2):
    (S, D), FF = x.shape, w1.shape[1]
    nd, nf = D // 128, FF // 128
    vmem = pltpu.VMEM

    def tiled(count, rows, dtype=U32, blocks=1):
        return vmem((blocks * -(-count // 4) * rows + SPARE, 512), dtype)

    def right(nk, nn):
        return tiled(7 * (nk // 2) * (nn // 2) + nk * nn - nk // 2 * 2 * (nn // 2 * 2), 64)

    left = 9 * (nd // 2) + 2
    stats = [vmem((TB + 32, 128), F32)] * 2
    pairs = [vmem((RB, 256), U32)] * (nd // 2 + 1)
    hbm = pl.BlockSpec(memory_space=pl.ANY)
    return pl.pallas_call(
        _kernel,
        in_specs=[hbm] * 5,
        out_specs=hbm,
        out_shape=jax.ShapeDtypeStruct((S, D), x.dtype),
        scratch_shapes=[
            vmem((S, D), BF), vmem((D, 3 * D), BF), vmem((D, D), BF), vmem((D, FF), BF), vmem((FF, D), BF),
            [right(nd, nd + i) for i in (0, -1, 1)], right(nd, nd), right(nd, nf), right(nf, nd), stats, stats,
            tiled(left, RH, blocks=2), vmem((2 * RB, 384), U32), pairs, [pairs] * 2,
            vmem((D // 2 + 16, TB), U32), vmem((S // TB * D // 2 + 16, TB), U32), vmem((S // 2 + 64, D), U32),
            vmem((S // 2 + SPARE, 128 * H), U32), vmem((S // TB * 24 * H + 16, TB), F32),
            [vmem((264, 512), F32)] * 2, [vmem((144 + SPARE, 512), U32)] * 2, [vmem((128, TB), F32)] * nd,
            tiled(left, RH), vmem((S, D), F32), tiled(left, RH), [tiled(9 * (nf // 2), RH)] * 2,
            vmem((S + 2 * SPARE, D), BF),
            pltpu.SemaphoreType.DMA((7,)), pltpu.SemaphoreType.DMA((4,)), pltpu.SemaphoreType.DMA((4,)),
        ],
        compiler_params=pltpu.CompilerParams(vmem_limit_bytes=100 << 20),
        name="fused_layer",
    )(x, wqkv, wo, w1, w2)


@jax.jit
def pallas_sequential_preLN__sliding_block__dense_activation_relu__prompt_kernel(
    A_x: jax.Array,
    A_wqkv: jax.Array,
    A_wo: jax.Array,
    B_x: jax.Array,
    B_w1: jax.Array,
    B_w2: jax.Array,
):
    del B_x
    return _layer(A_x.reshape(A_x.shape[-2:]), A_wqkv, A_wo, B_w1, B_w2).reshape(A_x.shape)
```
